```python
import os as _os
_os.environ.setdefault("JAX_PLATFORMS", "cpu")
import jax
import jax.numpy as jnp

def _softmax(x, axis=-1):
    return jax.nn.softmax(x, axis=axis)
def _gelu(x):
    return jax.nn.gelu(x, approximate=True)
def _silu(x):
    return jax.nn.silu(x)
def _sigmoid(x):
    return jax.nn.sigmoid(x)
def _layernorm(x, axis=-1, eps=1e-5):
    m = jnp.mean(x, axis=axis, keepdims=True)
    v = jnp.var(x, axis=axis, keepdims=True)
    return (x - m) / jnp.sqrt(v + eps)
def _scatter_add(tgt, idx, src, axis=0):
    return tgt.at[idx].add(src)
def _segment_sum(src, seg, n):
    return jax.ops.segment_sum(src, seg, n)
class _Rng:
    def __init__(self, key):
        self._k = key
    def _next(self):
        self._k, sub = jax.random.split(self._k)
        return sub
    def normal(self, shape):
        return jax.random.normal(self._next(), shape, dtype=jnp.bfloat16)
    def randint(self, lo, hi, shape):
        return jax.random.randint(self._next(), shape, lo, hi, dtype=jnp.int32)
    def uniform(self, shape, lo=0.0, hi=1.0):
        return jax.random.uniform(self._next(), shape, jnp.bfloat16, lo, hi)
    def permutation(self, n):
        return jax.random.permutation(self._next(), n)


kernel_name = 'parallel_sum__ssm_conv_s4__glu_gated_bilinear__prompt'

def setup_inputs():
    _rng = _Rng(jax.random.key(int.from_bytes(__import__("os").urandom(4), "little")))
    _w = (lambda a: (lambda t: t.astype(jnp.bfloat16) if jnp.issubdtype(t.dtype, jnp.floating) else t)(jnp.asarray(a)))
    def _A_setup():
        B, L, D, N = 1, 2048, 640, 192
        A_re = -jnp.exp((lambda *s: _rng.normal(s) * 0.1)(D, N))
        A_im = jnp.pi * (lambda *s: _rng.normal(s) * 0.1)(D, N)
        B_re = (lambda *s: _rng.normal(s) * 0.1)(D, N)
        B_im = (lambda *s: _rng.normal(s) * 0.1)(D, N)
        C_re = (lambda *s: _rng.normal(s) * 0.1)(D, N)
        C_im = (lambda *s: _rng.normal(s) * 0.1)(D, N)
        log_dt = (lambda *s: _rng.normal(s) * 0.1)(D) * 0.5 - 4.0
        Dskip = (lambda *s: _rng.normal(s) * 0.05)(D)
        return {
            "u": _w((lambda *s: _rng.normal(s) * 0.05)(B, L, D)),
            "A_re": _w(A_re),
            "A_im": _w(A_im),
            "B_re": _w(B_re),
            "B_im": _w(B_im),
            "C_re": _w(C_re),
            "C_im": _w(C_im),
            "log_dt": _w(log_dt),
            "Dskip": _w(Dskip),
        }
    _A_in = _A_setup()

    def _B_setup():
        B, S, D, F = 1, 2048, 640, 1536
        return {
            "x": _w((lambda *s: _rng.normal(s) * 0.05)(B, S, D)),
            "w_gate": _w((lambda *s: _rng.normal(s) * 0.05)(D, F) * (D ** -0.5)),
            "w_up": _w((lambda *s: _rng.normal(s) * 0.05)(D, F) * (D ** -0.5)),
            "w_down": _w((lambda *s: _rng.normal(s) * 0.05)(F, D) * (F ** -0.5)),
        }
    _B_in = _B_setup()

    return {
        "A_u": _A_in["u"],
        "A_A_re": _A_in["A_re"],
        "A_A_im": _A_in["A_im"],
        "A_B_re": _A_in["B_re"],
        "A_B_im": _A_in["B_im"],
        "A_C_re": _A_in["C_re"],
        "A_C_im": _A_in["C_im"],
        "A_log_dt": _A_in["log_dt"],
        "A_Dskip": _A_in["Dskip"],
        "B_x": _B_in["x"],
        "B_w_gate": _B_in["w_gate"],
        "B_w_up": _B_in["w_up"],
        "B_w_down": _B_in["w_down"],
    }

def reference(A_u, A_A_re, A_A_im, A_B_re, A_B_im, A_C_re, A_C_im, A_log_dt, A_Dskip, B_x, B_w_gate, B_w_up, B_w_down):
    def _A_ref(u, A_re, A_im, B_re, B_im, C_re, C_im, log_dt, Dskip):
        Bsz, L, D = u.shape
        dt = jnp.exp(log_dt)[:, None]
        A = A_re + 1j * A_im
        Bc = B_re + 1j * B_im
        Cc = C_re + 1j * C_im
        logdA = dt * A
        dB = dt * Bc
        l = (lambda x, dt: x.astype(dt))(jnp.arange(L), A_re.dtype)
        P = jnp.exp(logdA[:, :, None] * l[None, None, :])
        K = jnp.einsum("dn,dnl,dn->dl", Cc, P, dB).real
        L2 = 2 * L
        Kp = jnp.pad(K, ((0, 0), (0, L)))
        up = (lambda x, *d: x.transpose(*d))(u, 0, 2, 1)
        up = jnp.pad(up, ((0, 0), (0, 0), (0, L)))
        Kf = (lambda x, axes=(-2,-1): jnp.fft.rfft2(x.astype(jnp.float32), axes=axes))(Kp[:, None, :], axes=(-2, -1))
        Uf = (lambda x, axes=(-2,-1): jnp.fft.rfft2(x.astype(jnp.float32), axes=axes))(up[:, :, None, :], axes=(-2, -1))
        Yf = Uf * Kf[None, :, :, :]
        y = (lambda x, s, axes=(-2,-1): jnp.fft.irfft2(x, s=s, axes=axes).astype(jnp.bfloat16))(Yf, (1, L2), axes=(-2, -1))[:, :, 0, :L]
        y = (lambda x, *d: x.transpose(*d))(y, 0, 2, 1) + u * Dskip[None, None, :]
        return y

    def _B_ref(x, w_gate, w_up, w_down):
        g = jnp.einsum("bsd,df->bsf", x, w_gate)
        u = jnp.einsum("bsd,df->bsf", x, w_up)
        h = g * u
        return jnp.einsum("bsf,fd->bsd", h, w_down)

    x = A_u
    xn = _layernorm(x, axis=-1)
    return x + _A_ref(xn, A_A_re, A_A_im, A_B_re, A_B_im, A_C_re, A_C_im, A_log_dt, A_Dskip) + _B_ref(xn, B_w_gate, B_w_up, B_w_down)
```

```python
import functools
import os
import numpy as np
import jax
import jax.numpy as jnp
import jax.experimental.pallas as pl
import jax.experimental.pallas.tpu as pltpu

L, D, N, F = 2048, 640, 192, 1536
T = 128
NB = L // T
NCT = D // 128
RB = 256
NS = L // RB
OCT = D // 8 // NS
FC = 256
f32, bf16, u32, i32 = jnp.float32, jnp.bfloat16, jnp.uint32, jnp.int32
ONLY = os.environ.get("ONLY")
NCH = int(os.environ.get("NCH", "2"))
XL = int(os.environ.get("XL", "1"))


def _tile_lags():
    lane = np.arange(128)
    q, k = lane // 4, lane % 4
    j = q // 2 + 16 * (q % 2)
    t = [1 + lane, 129 + lane]
    for a in ([258, 260, 262, 264], [516, 772, 520, 776], [1544, 1800, 1032, 1288]):
        t.append(np.asarray(a)[k] + 8 * j)
    return np.stack(t)


def _pack_np(a):
    b = np.asarray(a, np.float32).astype(jnp.bfloat16).view(np.uint16).astype(np.uint32)
    return b[0::2] | (b[1::2] << 16)


@functools.lru_cache(maxsize=None)
def _consts():
    rl = np.arange(L).astype(np.float32).astype(jnp.bfloat16).astype(np.int64)
    lags = _tile_lags()
    where = {int(v): (t, l) for t in range(5) for l, v in enumerate(lags[t])}
    kk = np.arange(128) + 0.5
    mats = {}
    for m in range(NB):
        for p in range(1, 256):
            lag = 128 * (m - 1) + p
            if lag <= 0 or lag >= L:
                continue
            t, l = where[int(rl[lag])]
            M = mats.setdefault((t, m), np.zeros((256, 128)))
            ang = -2 * np.pi * kk * p / 256
            re, im = np.cos(ang), np.sin(ang)
            M[:128, l] += im - re
            M[128:, l] += -(re + im)
    keys = sorted(mats)
    fk = np.concatenate([mats[k] for k in keys], axis=0)
    s = np.arange(128)
    ang = -2 * np.pi * kk[:, None] * s[None, :] / 256
    fu = np.concatenate([np.cos(ang), np.sin(ang)], axis=0)
    th = 2 * np.pi * kk[None, :] * (128 + s[:, None]) / 256
    fi = np.concatenate([np.cos(th) / 128.0, -np.sin(th) / 128.0], axis=0)
    small = np.concatenate([np.zeros((8, 128), np.uint32), _pack_np(fu), _pack_np(fi)], axis=0)
    return keys, _pack_np(fk), small


def _pk(x):
    return pltpu.bitcast(x.astype(bf16), u32)


def _upk(x):
    return pltpu.bitcast(x, bf16)


def _nt(a, b):
    return jax.lax.dot_general(a, b, (((1,), (1,)), ((), ())), preferred_element_type=f32)


def _dot(a, b):
    return jnp.dot(a, b, preferred_element_type=f32)


def _cis(mag, th):
    kf = jnp.floor(th * (2.0 / np.pi) + 0.5)
    k = kf.astype(i32)
    r = ((th - kf * 1.5703125) - kf * 4.837512969970703125e-4) - kf * 7.54978995489188216e-8
    r = jnp.minimum(jnp.maximum(r, -1.0), 1.0)
    r2 = r * r
    s = r + r * (r2 * (-1.6666654611e-1 + r2 * (8.3321608736e-3 + r2 * -1.9515295891e-4)))
    c = 1.0 + r2 * (-0.5 + r2 * (4.166664568298827e-2 + r2 * (-1.388731625493765e-3 + r2 * 2.443315711809948e-5)))
    swap = (k & 1) == 1
    mb = pltpu.bitcast(mag, i32)
    ms = pltpu.bitcast(mb ^ ((k & 2) << 30), f32)
    mc = pltpu.bitcast(mb ^ (((k + 1) & 2) << 30), f32)
    return mc * jnp.where(swap, s, c), ms * jnp.where(swap, c, s)


def _kernel(x_hbm, are_h, aim_h, bre_h, bim_h, cre_h, cim_h, ldt_h, dsk_h, wg_h, wu_h, wd_h,
            fk_h, sm_h, fl_h, o_hbm,
            x_v, par_v, ldt_v, dsk_v, wg_v, wu_v, wd_v, fk_v, sm_v, coef_s, zw_s, xn_s, h_s, u_s,
            xs_s, es_s, kc_s, kw_s, y_s, o_s, fl_s, sems):
    keys = _consts()[0]
    never_src = sm_v
    x_v, wg_v, wu_v, wd_v, xn_s, h_s, xs_s, es_s, y_s, o_s = [
        r.bitcast(bf16) for r in (x_v, wg_v, wu_v, wd_v, xn_s, h_s, xs_s, es_s, y_s, o_s)]

    def cp(a, b, i):
        return pltpu.make_async_copy(a, b, sems.at[i])

    c_par = [cp(p, par_v.at[i], i) for i, p in enumerate((are_h, aim_h, bre_h, bim_h, cre_h, cim_h))]
    c_ldt, c_dsk, c_sm = cp(ldt_h, ldt_v, 6), cp(dsk_h, dsk_v, 7), cp(sm_h, sm_v, 8)
    c_wg, c_wu, c_fk = cp(wg_h, wg_v, 10), cp(wu_h, wu_v, 11), cp(fk_h, fk_v, 13)
    c_out = [cp(o_s.at[:, ct * 128:(ct + 1) * 128], o_hbm.at[:, ct * 128:(ct + 1) * 128], 14 + ct) for ct in range(NCT)]
    c_x = [cp(x_hbm.at[t * RB:(t + 1) * RB], x_v.at[t * RB:(t + 1) * RB], 19 + t) for t in range(NS)]
    c_wd = [cp(wd_h.at[:, ct * 128:(ct + 1) * 128], wd_v.at[:, ct * 128:(ct + 1) * 128], 27 + ct) for ct in range(NCT)]
    c_fl = cp(fl_h, fl_s, 32)

    class Ctx:
        pass

    def mk(paced=True):
        c = Ctx()
        c.lane = jax.lax.broadcasted_iota(i32, (8, 128), 1)
        c.sub = jax.lax.broadcasted_iota(i32, (8, 128), 0)
        c.never = never_src[0:8, :] != 0
        c.tok = None
        c.paced = paced
        return c

    def tie(c, v, tok):
        if tok is None or not c.paced:
            return v
        if v.shape == (8, 128):
            return jnp.where(c.never, tok, v)
        return jnp.concatenate([jnp.where(c.never, tok, v[:, :128]), v[:, 128:]], axis=1)

    def cmul(a, b):
        return a[0] * b[0] - a[1] * b[1], a[0] * b[1] + a[1] * b[0]

    def csq(a):
        return a[0] * a[0] - a[1] * a[1], (a[0] + a[0]) * a[1]

    def a0(c, ct):
        cs = slice(ct * 128, (ct + 1) * 128)
        dt = jnp.exp(ldt_v[...].astype(f32).reshape(1, D)[:, cs]).astype(bf16).astype(f32)
        outs = [[], [], [], []]
        k0 = None
        toks = [c.tok, c.tok]
        for i in range(N // 8):
            ld = lambda q: par_v[q, 8 * i:8 * i + 8, cs].astype(f32)
            th = tie(c, dt * ld(1), toks[i % 2])
            zr, zi = _cis(jnp.exp(dt * ld(0)), th)
            cb = cmul((ld(4), ld(5)), (tie(c, ld(2), toks[i % 2]), tie(c, ld(3), toks[i % 2])))
            wr, wi = dt * cb[0], dt * cb[1]
            k0 = wr if k0 is None else k0 + wr
            toks[i % 2] = zr
            for o, v in zip(outs, (zr, zi, wr, wi)):
                o.append(v)
        c.tok = toks[1]
        coef_s[:, cs] = jnp.broadcast_to(
            jnp.sum(k0, axis=0, keepdims=True) + dsk_v[...].astype(f32).reshape(1, D)[:, cs], (8, 128))
        hi = [outs[0][16:] * 2, outs[1][16:] * 2, [-v for v in outs[3][16:]] + outs[2][16:], outs[2][16:] + outs[3][16:]]
        for q in range(4):
            zw_s[q, cs, 0:128] = jnp.concatenate(outs[q][:16], axis=0).T
            zw_s[q, cs, 128:256] = jnp.concatenate(hi[q], axis=0).T

    def ln(c, t):
        toks = [c.tok] * 4
        for i in range(RB // 16):
            r0 = t * RB + 16 * i
            x = x_v[r0:r0 + 16, :].astype(f32)
            halves = []
            for hh in range(2):
                xx = tie(c, x[8 * hh:8 * hh + 8], toks[(2 * i + hh) % 4])
                mu = jnp.sum(xx, axis=1, keepdims=True) * (1.0 / D)
                xc = xx - mu
                var = jnp.sum(xc * xc, axis=1, keepdims=True) * (1.0 / D)
                xn = xc * jax.lax.rsqrt(var + 1e-5)
                toks[(2 * i + hh) % 4] = xn[:, :128]
                halves.append(xn)
            xn_s[r0:r0 + 16, :] = jnp.concatenate(halves, axis=0).astype(bf16)
        c.tok = toks[3]

    def xe_octet(c, o, slot):
        lo64 = c.lane < 64
        slo = jnp.concatenate([c.sub < 4] * 2, axis=1)
        r0 = 8 * o

        def mix(a, b):
            ra = pltpu.roll(a, 4, 0)
            rb = ra if b is a else pltpu.roll(b, 4, 0)
            return jnp.where(slo, a, rb), jnp.where(slo, ra, b)

        def mixc(a, b):
            r = [mix(u, v) for u, v in zip(a, b)]
            return (r[0][0], r[1][0]), (r[0][1], r[1][1])

        def part(v, h):
            return v[0][:, 128 * h:128 * h + 128], v[1][:, 128 * h:128 * h + 128]

        def cmulc(a, b):
            return a[0] * b[0] + a[1] * b[1], a[1] * b[0] - a[0] * b[1]

        def tiec(s, tok):
            return tuple(tie(c, v, tok) for v in s)

        def put(ref, g, lst, h):
            b0 = (slot * 2 * OCT + g) * 8 * len(lst)
            for i in range(0, len(lst), 2):
                cols = [(0, 0), (1, 1)] if h == 0 else [(1, 2)]
                for q, cb in cols:
                    v = jnp.concatenate([lst[i][q], lst[i + 1][q]], axis=0)
                    ref[b0 + 8 * i:b0 + 8 * i + 16, 128 * cb:128 * cb + 128] = v.astype(bf16)

        def tie2(v):
            if c.tok is None or not c.paced:
                return v
            return jnp.concatenate([jnp.where(c.never, c.tok, v[:, :128]), jnp.where(c.never, c.tok, v[:, 128:])], axis=1)

        z = (tie2(zw_s[0, r0:r0 + 8, :]), tie2(zw_s[1, r0:r0 + 8, :]))
        w = (zw_s[2, r0:r0 + 8, :], zw_s[3, r0:r0 + 8, :])
        pw = {1: z}
        e = 1
        while e < 512:
            pw[2 * e] = csq(pw[e])
            e *= 2
        wz = cmul(w, z)
        wz5 = cmul(wz, pw[4])
        p772 = cmul(cmul(pw[512], pw[256]), pw[4])
        x0 = mixc(wz, wz5)
        m1 = mixc(z, z)
        m256 = mixc(pw[256], pw[256])
        mm = mixc(p772, pw[256])
        m8 = mixc(pw[8], pw[8])
        l01 = jnp.where(lo64, 1.0, 0.0).astype(f32)
        one = (jnp.concatenate([jnp.ones((8, 128), f32), 1.0 - l01], axis=1),
               jnp.concatenate([jnp.zeros((8, 128), f32), l01], axis=1))
        er, ei = pw[128]
        eb = (jnp.concatenate([er[:, :128], jnp.where(lo64, ei[:, 128:], er[:, 128:])], axis=1),
              jnp.concatenate([-ei[:, :128], jnp.where(lo64, er[:, 128:], -ei[:, 128:])], axis=1))
        e0 = mixc(one, eb)
        toks = [p772[0][:, :128]] * XL
        seg = 0
        for g in range(2):
            for h in range(2):
                a1, a256, am, a8 = part(m1[g], h), part(m256[g], h), part(mm[g], h), part(m8[g], h)
                xs = [tiec(part(x0[g], h), toks[seg % XL])]
                for _ in range(3):
                    xs.append(cmul(xs[-1], a1))
                xs.append(cmul(xs[1], a256))
                xs.append(cmul(xs[3], a256))
                xs.append(cmul(xs[5], a256))
                xs.append(cmul(xs[6], a256))
                xs.append(cmul(xs[7], am))
                xs.append(cmul(xs[8], a256))
                put(xs_s, 2 * (o % OCT) + g, xs, h)
                es = [tiec(part(e0[g], h), xs[-1][1])]
                for _ in range(15):
                    es.append(cmulc(es[-1], a8))
                put(es_s, 2 * (o % OCT) + g, es, h)
                toks[seg % XL] = es[-1][1]
                seg += 1
        c.tok = toks[(seg - 1) % XL]

    def xe(c, b):
        for o in range(b * OCT, (b + 1) * OCT):
            xe_octet(c, o, b % 2)

    def c2(c, ct):
        slot = ct % 2
        chain = [c.tok] * NCH
        cnt = 0
        for p2 in range(8):
            res = [[None] * 2 for _ in range(2)]
            for hh in range(2):
                rws = slice(p2 * 16 + hh * 8, p2 * 16 + hh * 8 + 8)
                k1 = None
                for s in range(3):
                    U = [u_s[ct, s, j, rws, :] for j in range(NB)]
                    K = [kw_s[slot, s, j, rws, :] for j in range(NB)]
                    out = []
                    for i in range(NB):
                        a = k1[i] if s else K[0] * U[i]
                        a = tie(c, a, chain[cnt % NCH])
                        for m in range(0 if s else 1, i + 1):
                            a = a + K[m] * U[i - m]
                        chain[cnt % NCH] = a
                        cnt += 1
                        out.append(a)
                    if s == 0:
                        k1 = out
                    else:
                        res[2 - s][hh] = out
            for part in range(2):
                for i in range(NB):
                    v = jnp.concatenate([res[part][0][i], res[part][1][i]], axis=0)
                    y_s[slot * 256 + part * 128 + p2 * 16:slot * 256 + part * 128 + p2 * 16 + 16, i * 128:(i + 1) * 128] = v.astype(bf16)

    def ffn1(t, fc):
        xn = xn_s[t * RB:(t + 1) * RB, :]
        g = _dot(xn, wg_v[:, fc * FC:(fc + 1) * FC])
        u = _dot(xn, wu_v[:, fc * FC:(fc + 1) * FC])
        h_s[t * RB:(t + 1) * RB, fc * FC:(fc + 1) * FC] = (g * u).astype(bf16)

    def ufwd(j):
        xn = xn_s[j * T:(j + 1) * T, :]
        uf = _dot(_upk(sm_v[8:136, :]), xn)
        for ct in range(NCT):
            a_ = uf[:128, ct * 128:(ct + 1) * 128]
            b_ = uf[128:, ct * 128:(ct + 1) * 128]
            u_s[ct, 0, j] = (a_ + b_) * (-0.5)
            u_s[ct, 1, j] = a_
            u_s[ct, 2, j] = b_

    def kmm_octet(c, o):
        slot = (o // OCT) % 2
        lane, sub = c.lane, c.sub
        slo = sub < 4
        gi = [slot * 2 * OCT + 2 * (o % OCT) + g for g in range(2)]
        res = [_nt(xs_s[80 * q:80 * q + 80, :], es_s[128 * q:128 * q + 128, :]) for q in gi]
        dk = (lane - sub) & 3

        def merge(r, vs):
            out = None
            for k in reversed(range(len(vs))):
                src = r[8 * vs[k]:8 * vs[k] + 8, :]
                if k:
                    src = pltpu.roll(src, k, 1)
                out = src if out is None else jnp.where(dk == k, src, out)
            return out

        def derot(x):
            x = jnp.where((sub & 1) == 1, pltpu.roll(x, 127, 1), x)
            return jnp.where((sub & 2) == 2, pltpu.roll(x, 126, 1), x)

        def pair(vs):
            a, b = merge(res[0], vs), merge(res[1], vs)
            return derot(jnp.where(slo, a, pltpu.roll(b, 4, 0))), derot(jnp.where(slo, pltpu.roll(a, 4, 0), b))

        a, b = pair([0, 1, 2, 3])
        l8 = (lane & 7) < 4
        l4 = (lane & 3) < 2
        t0 = jnp.where(l8, a, pltpu.roll(b, 4, 1))
        t1 = jnp.where(l8, pltpu.roll(a, 124, 1), b)
        a, b = pair([4, 5, 6, 7])
        t2 = jnp.where(l4, a, pltpu.roll(b, 2, 1))
        t3 = jnp.where(l4, pltpu.roll(a, 126, 1), b)
        a, b = pair([8, 9])
        t4 = jnp.where(l4, a, pltpu.roll(b, 2, 1))
        for i, t in enumerate((t0, t1, t2, t3, t4)):
            kc_s[i, 8 * o:8 * o + 8, :] = t

    def kfwd(ct):
        cs = slice(ct * 128, (ct + 1) * 128)
        slot = ct % 2
        acc = {}
        last = {m: max(tt for (tt, mm) in keys if mm == m) for m in range(NB)}
        for pos, (tau, m) in enumerate(keys):
            kt = kc_s[tau, cs, :].astype(bf16)
            v = _nt(_upk(fk_v[pos * 128:(pos + 1) * 128, :]), kt)
            acc[m] = v if m not in acc else acc[m] + v
            if last[m] == tau:
                e_, f_ = acc[m][:128], acc[m][128:]
                kw_s[slot, 0, m] = e_ + f_
                kw_s[slot, 1, m] = e_
                kw_s[slot, 2, m] = f_

    def fin(ct, rb):
        cs = slice(ct * 128, (ct + 1) * 128)
        slot = ct % 2
        r0 = rb * RB
        dn = _dot(h_s[r0:r0 + RB, :], wd_v[:, cs])
        fi = jnp.concatenate([_upk(sm_v[136:200, :]), _upk(sm_v[200:264, :])], axis=1)
        yt = _dot(fi, y_s[slot * 256:slot * 256 + 256, r0:r0 + RB])
        y = jnp.concatenate([yt[:, i * 128:(i + 1) * 128] for i in range(RB // T)], axis=0)
        xn = xn_s[r0:r0 + RB, cs].astype(f32)
        o = x_v[r0:r0 + RB, cs].astype(f32) + xn * coef_s[0:1, cs] + y + dn
        o_s[r0:r0 + RB, cs] = o.astype(bf16)

    def prologue():
        for cc in [c_fl, c_sm, c_ldt, c_dsk] + c_par + c_x[:2] + [c_wg, c_wu] + c_x[2:] + [c_fk] + c_wd:
            cc.start()
        for cc in [c_fl, c_sm, c_ldt, c_dsk] + c_par:
            cc.wait()
        c = mk(paced=False)
        a0(c, 0)
        xe(c, 0)
        c_x[0].wait()
        c_x[1].wait()
        ln(c, 0)
        ln(c, 1)
        c_wg.wait()
        c_wu.wait()

    a0_at = {0: 1, 2: 2, 3: 3, 5: 4}
    ln_at = {0: [2], 1: [3], 2: [4], 3: [5], 4: [6], 5: [7]}
    uf_at = {0: [0, 1, 2, 3], 1: [4, 5], 2: [6, 7], 3: [8, 9], 4: [10, 11], 5: [12, 13], 6: [14, 15]}
    kf_at = {6: 0, 7: 1}

    def s_step(t):
        def run():
            if t < 6:
                c_x[t + 2].wait()
            elif t == 6:
                c_fk.wait()
            c = mk()
            for o in range(t * OCT, (t + 1) * OCT):
                kmm_octet(c, o)
            for j in uf_at.get(t, []):
                ufwd(j)
            if t in kf_at:
                kfwd(kf_at[t])
            for fc in range(F // FC):
                ffn1(t, fc)
            if t in a0_at:
                a0(c, a0_at[t])
            if t + 1 < NS:
                xe(c, t + 1)
            else:
                c2(c, 0)
            for tt in ln_at.get(t, []):
                ln(c, tt)
        return run

    def q_step(ct):
        def run():
            c_wd[ct].wait()
            if ct > 0:
                c_out[ct - 1].start()
            c = mk()
            if ct + 2 < NCT:
                kfwd(ct + 2)
            for rb in range(NS):
                fin(ct, rb)
            if ct + 1 < NCT:
                c2(c, ct + 1)
            if ct == NCT - 1:
                c_out[ct].start()
                for cc in c_out:
                    cc.wait()
        return run

    steps = [prologue] + [s_step(t) for t in range(NS)] + [q_step(ct) for ct in range(NCT)]
    steps[0]()
    for i, fn in enumerate(steps[1:]):
        pl.when(fl_s[i] == 0)(fn)


@jax.jit
def pallas_parallel_sum__ssm_conv_s4__glu_gated_bilinear__prompt_kernel(A_u, A_A_re, A_A_im, A_B_re, A_B_im, A_C_re, A_C_im, A_log_dt, A_Dskip, B_x, B_w_gate, B_w_up, B_w_down):
    keys, fk, small = _consts()
    hbm = pl.BlockSpec(memory_space=pltpu.HBM)
    out = pl.pallas_call(
        _kernel,
        in_specs=[hbm] * 15,
        out_specs=hbm,
        out_shape=jax.ShapeDtypeStruct((L, D), bf16),
        scratch_shapes=[
            pltpu.VMEM((L // 2, D), u32),
            pltpu.VMEM((6, N, D), bf16),
            pltpu.VMEM((D,), bf16), pltpu.VMEM((D,), bf16),
            pltpu.VMEM((D // 2, F), u32), pltpu.VMEM((D // 2, F), u32), pltpu.VMEM((F // 2, D), u32),
            pltpu.VMEM(fk.shape, u32), pltpu.VMEM(small.shape, u32),
            pltpu.VMEM((8, D), f32),
            pltpu.VMEM((4, D, 256), f32),
            pltpu.VMEM((L // 2, D), u32),
            pltpu.VMEM((L // 2, F), u32),
            pltpu.VMEM((NCT, 3, NB, 128, 128), f32),
            pltpu.VMEM((2 * 2 * OCT * 40, 384), u32),
            pltpu.VMEM((2 * 2 * OCT * 64, 384), u32),
            pltpu.VMEM((5, D, 128), f32),
            pltpu.VMEM((2, 3, NB, 128, 128), f32),
            pltpu.VMEM((2 * 128, L), u32),
            pltpu.VMEM((L // 2, D), u32),
            pltpu.SMEM((32,), i32),
            pltpu.SemaphoreType.DMA((34,)),
        ],
        compiler_params=pltpu.CompilerParams(vmem_limit_bytes=100 * 1024 * 1024),
    )(A_u.reshape(L, D), A_A_re.T, A_A_im.T, A_B_re.T, A_B_im.T, A_C_re.T, A_C_im.T, A_log_dt, A_Dskip,
      B_w_gate, B_w_up, B_w_down, jnp.asarray(fk), jnp.asarray(small), jnp.zeros((32,), i32))
    return out.reshape(1, L, D)
```

```python
import functools
import os
import numpy as np
import jax
import jax.numpy as jnp
import jax.experimental.pallas as pl
import jax.experimental.pallas.tpu as pltpu

L, D, N, F = 2048, 640, 192, 1536
RB = 256
NS = L // RB
NCT = D // 128
NCK = 6
XR = 72
f32, bf16, u32, i32 = jnp.float32, jnp.bfloat16, jnp.uint32, jnp.int32
ONLYB = os.environ.get("ONLYB")
CFG = dict(kv.split("=") for kv in os.environ.get("CFG", "").split(",") if kv)
cfg = lambda k, d: int(CFG.get(k, d))

_PARTS = [(4, 2, 256, 512), (4, 3, 0, 512), (4, 4, 0, 256), (8, 4, 256, 512), (8, 5, 0, 512), (8, 6, 0, 512), (8, 7, 0, 512)]
_SEL = {1: [256], 2: [512], 3: [768, 1024], 4: [1280, 1536, 1792, 2048]}
_KD = {}
for _p in _PARTS:
    for _n, _w in [(q, 16 // _p[0]) for q in range(6)] + [("a+b", 1), ("a-b", 1), ("b", 1)]:
        _KD[_p, _n] = _KD.get("n", 0)
        _KD["n"] = _KD.get("n", 0) + _w


def _tile_lags():
    lane = np.arange(128)
    q, k = lane // 4, lane % 4
    j8 = 8 * (q // 2 + 16 * (q % 2))
    t = []
    for a0, a1, sh in (([1, 2, 3, 4], [5, 6, 7, 8], 1), ([258, 260, 516, 772], [262, 264, 520, 776], 2),
                       ([1544, 1800, 0, 0], [1032, 1288, 0, 0], 2)):
        a, b = np.asarray(a0)[k] + j8, np.roll(np.asarray(a1)[k] + j8, sh)
        m = lane % (2 * sh) < sh
        t += [np.where(m, a, b), np.where(m, b, a)]
    return np.stack(t[:5])


def _pack_np(a):
    b = np.asarray(a, np.float32).astype(jnp.bfloat16).view(np.uint16).astype(np.uint32)
    return b[0::2] | (b[1::2] << 16)


@functools.lru_cache(maxsize=None)
def _consts():
    rl = np.arange(L).astype(np.float32).astype(jnp.bfloat16).astype(np.int64)
    lags = _tile_lags()
    where = {int(v): (t, l) for t in range(5) for l, v in enumerate(lags[t])}
    r2 = 2 * np.arange(64)
    th = 2 * np.pi * (np.concatenate([r2, 127 - r2, 255 - r2, 128 + r2]) + 0.5) / 512

    def ef(p):
        re, im = np.cos(th * p).reshape(4, 64), -np.sin(th * p).reshape(4, 64)
        return np.stack([im - re, -(re + im)], axis=1).reshape(512)

    rows, off, hf = [], {}, []

    def add(key, m):
        off[key] = sum(x.shape[0] for x in rows)
        rows.append(m)

    for t in (0, 1):
        add(("B0", t), np.stack([ef(p)[:256] for p in lags[t]], axis=1))
    m = np.zeros((512, 128))
    for p in range(2, 257):
        tt, l = where[int(rl[256 + p])]
        assert tt == 2
        m[:, l] += ef(p) * (0.5 if p == 256 else 1.0)
    add("B1", m)
    assert rl[257] == 256
    hf.append(ef(1))
    for tau, lg in _SEL.items():
        parts = [p for p in _PARTS if p[0] == {3: 4, 4: 8}.get(tau)]
        blk = []
        for st, w, p0, p1 in parts:
            nr = 128 // st
            dm = np.zeros((4 * nr, 128))
            for pc in range(p0, p1 + 1, st):
                lag, odd = 256 * (w - 1) + pc, (pc // st) % 2
                assert all(int(rl[lag + d]) == lag for d in range(odd - st // 2, st // 2 + 1 - odd)
                           if p0 < pc + d < p1 and lag + d < L)
                tt, l = where[lag]
                if tt != tau:
                    assert pc == p0
                    continue
                v = ef(pc) * (0.5 if pc in (p0, p1) else 1.0)
                dm[2 * nr * odd:2 * nr * odd + nr, l] += v[0:nr]
                dm[2 * nr * odd + nr:2 * nr * odd + 2 * nr, l] += v[64:64 + nr]
            blk.append(dm)
        sel = np.zeros((16 * ((len(lg) + 1) // 2), 128))
        for j, lag in enumerate(lg):
            assert where[lag][0] == tau
            sel[8 * j:8 * j + 8, where[lag][1]] = 1.0
        add(("D", tau), np.concatenate([sel] + blk, axis=0))
        off["Dn", tau] = rows[-1].shape[0]
    for st in (4, 8):
        ho = 1 + 2 * sum(np.cos(th * d) for d in range(1, st // 2))
        off["T", st] = sum(x.shape[0] for x in hf)
        hf += [ho + 2 * np.cos(th * (st // 2)), ho * (-1.0) ** ((np.arange(256) % 64) // (128 // st)),
               sum(np.sin(th * d) for d in range(1, st // 2 + 1))]
    pos = np.arange(128)
    tc = th[8 * (pos // 16) + pos % 8]
    for c in range(4):
        a = tc[None, :] * (256 + 4 * np.arange(64) + c)[:, None]
        add(("I", c), np.where(pos[None, :] % 16 < 8, np.cos(a), -np.sin(a)) / 256.0)
    fk = _pack_np(np.concatenate(rows, axis=0))
    off["F32"] = fk.shape[0]
    hf = np.repeat(np.concatenate(hf)[:, None], 128, axis=1).astype(np.float32)
    big = np.concatenate([fk, hf.view(np.uint32)], axis=0)
    fu = []
    for par in range(2):
        a = th[:128, None] * (2 * pos + par)[None, :]
        fu.append(_pack_np(np.concatenate([np.cos(a), -np.sin(a)], axis=0)))
    zero = np.zeros((8, 128), np.uint32)
    small = np.concatenate([zero, zero, np.broadcast_to(np.arange(128) < 64, (8, 128)).astype(np.uint32),
                            np.broadcast_to(np.arange(8)[:, None] < 4, (8, 128)).astype(np.uint32)] + fu, axis=0)
    return off, big, small


class _Packed:
    def __init__(self, ref):
        self.ref = ref

    def __getitem__(self, idx):
        return pltpu.bitcast(self.ref[idx[0].start // 2:idx[0].stop // 2, idx[1]], bf16)

    def __setitem__(self, idx, v):
        self.ref[idx[0].start // 2:idx[0].stop // 2, idx[1]] = pltpu.bitcast(v.astype(bf16), u32)


class _Words:
    def __init__(self, ref):
        self.ref = ref

    def __getitem__(self, idx):
        return pltpu.bitcast(self.ref[2 * idx[0].start:2 * idx[0].stop, idx[1]], u32)

    def __setitem__(self, idx, v):
        self.ref[2 * idx[0].start:2 * idx[0].stop, idx[1]] = pltpu.bitcast(v, bf16)


class _Ctx:
    pass


def _nt(a, b):
    return jax.lax.dot_general(a, b, (((1,), (1,)), ((), ())), preferred_element_type=f32)


def _dot(a, b):
    return jnp.dot(a, b, preferred_element_type=f32)


def _cat(xs, axis):
    return jnp.concatenate(xs, axis=axis)


def _zip2(a, b):
    return pltpu.pack_elementwise([a, b], packed_dtype=bf16)


def _even_odd(w):
    return pltpu.bitcast(w << 16, f32), pltpu.bitcast(w & jnp.uint32(0xFFFF0000), f32)


def _cis(mag, th):
    kf = jnp.floor(th * (2.0 / np.pi) + 0.5)
    k = kf.astype(i32)
    r = ((th - kf * 1.5703125) - kf * 4.837512969970703125e-4) - kf * 7.54978995489188216e-8
    r = jnp.minimum(jnp.maximum(r, -1.0), 1.0)
    r2 = r * r
    s = r + r * (r2 * (-1.6666654611e-1 + r2 * (8.3321608736e-3 + r2 * -1.9515295891e-4)))
    c = 1.0 + r2 * (-0.5 + r2 * (4.166664568298827e-2 + r2 * (-1.388731625493765e-3 + r2 * 2.443315711809948e-5)))
    swap = (k & 1) == 1
    mb = pltpu.bitcast(mag, i32)
    ms = pltpu.bitcast(mb ^ ((k & 2) << 30), f32)
    mc = pltpu.bitcast(mb ^ (((k + 1) & 2) << 30), f32)
    return mc * jnp.where(swap, s, c), ms * jnp.where(swap, c, s)


def _cmul(a, b):
    return a[0] * b[0] - a[1] * b[1], a[0] * b[1] + a[1] * b[0]


def _cmulc(a, b):
    return a[0] * b[0] + a[1] * b[1], a[1] * b[0] - a[0] * b[1]


def _csq(a):
    return a[0] * a[0] - a[1] * a[1], (a[0] + a[0]) * a[1]


def tl(i, n=1):
    return slice(128 * i, 128 * (i + n))


def rs(a, n):
    return slice(a, a + n)


def _kernel(x_hbm, are_h, aim_h, bre_h, bim_h, cre_h, cim_h, ldt_h, dsk_h, wg_h, wu_h, wd_h,
            big_h, sm_h, o_hbm,
            x_v, par_v, ldt_v, dsk_v, wg_v, wu_v, wd_v, big_v, sm_v, coef_s, zw_s, xn_u, xa_u, ha_u,
            wt_u, wdt_u, u_s, xs_u, es_u, kc_s, kw_s, kd_s, y_u, o_s, dum_v, sems):
    off = _consts()[0]
    xn_s, xa_s, ha_s, wt_s, wdt_s, xs_s, es_s, y_s, big_s, sm_s = [
        _Packed(r) for r in (xn_u, xa_u, ha_u, wt_u, wdt_u, xs_u, es_u, y_u, big_v, sm_v)]
    x_u, wg_u, wu_u, wd_u, o_u = [_Words(r) for r in (x_v, wg_v, wu_v, wd_v, o_s)]
    AL = slice(None)
    nsem = [0]

    def grp(pairs):
        nsem[0] += 1
        return [pltpu.make_async_copy(a, b, sems.at[nsem[0] - 1]) for a, b in pairs]

    def cf(r0, n):
        return pltpu.bitcast(big_v[rs(off["F32"] + r0, n), :], f32)

    def mk(paced=True):
        c = _Ctx()
        c.never = (sm_v[0:8, :] != 0) if paced else None
        c.tok = c.xt = None
        c.cnt = 0
        return c

    def tie(c, v, tok):
        if tok is None or c.never is None:
            return v
        if tok.dtype != v.dtype:
            tok = pltpu.bitcast(tok, v.dtype)
        h = jnp.where(c.never, tok, v[:, :128])
        return h if v.shape[1] == 128 else _cat([h, v[:, 128:]], 1)

    def a0(c, ct, nc):
        cs = tl(ct)
        dt = jnp.exp(ldt_v[...].astype(f32).reshape(1, D)[:, cs]).astype(bf16).astype(f32)
        outs = [[], [], [], []]
        k0 = None
        toks = [c.tok] * nc
        for i in range(N // 8):
            ld = lambda q: par_v[q, 8 * i:8 * i + 8, cs].astype(f32)
            tk = toks[i % nc]
            zr, zi = _cis(jnp.exp(dt * ld(0)), tie(c, dt * ld(1), tk))
            cb = _cmul((ld(4), ld(5)), (tie(c, ld(2), tk), tie(c, ld(3), tk)))
            wr, wi = dt * cb[0], dt * cb[1]
            k0 = wr if k0 is None else k0 + wr
            toks[i % nc] = zr
            for o, v in zip(outs, (zr, zi, wr, wi)):
                o.append(v)
        c.tok = toks[-1]
        coef_s[:, cs] = jnp.broadcast_to(
            jnp.sum(k0, axis=0, keepdims=True) + dsk_v[...].astype(f32).reshape(1, D)[:, cs], (8, 128))
        hi = [outs[0][16:] * 2, outs[1][16:] * 2, [-v for v in outs[3][16:]] + outs[2][16:], outs[2][16:] + outs[3][16:]]
        for q in range(4):
            for h, v in enumerate((_cat(outs[q][:16], 0).T, _cat(hi[q], 0).T)):
                zw_s[q, cs, tl(h)] = v
                c.xt = v[120:128] if c.xt is None else c.xt + v[120:128]

    def ln(c, t, toks):
        for i in range(8):
            eo = ([], [])
            for g in range(2):
                wr = rs(128 * t + 16 * i + 8 * g, 8)
                for hh, xx in enumerate(_even_odd(x_u[wr, AL])):
                    ci = (4 * i + 2 * g + hh) % len(toks)
                    xx = tie(c, xx, toks[ci])
                    mu = jnp.sum(xx, axis=1, keepdims=True) * (1.0 / D)
                    var = jnp.maximum(jnp.sum(xx * xx, axis=1, keepdims=True) * (1.0 / D) - mu * mu, 0.0)
                    if c.never is not None:
                        xx = pltpu.unpack_elementwise(x_u[wr, AL], index=hh, packed_dtype=bf16, unpacked_dtype=f32)
                    xn = (xx - mu) * jax.lax.rsqrt(var + 1e-5)
                    toks[ci] = xn[:, :128]
                    eo[hh].append(xn)
            top, bot = _cat(eo[0], 0), _cat(eo[1], 0)
            xn_s[rs(RB * t + 16 * i, 16), AL] = top
            xn_s[rs(RB * t + 128 + 16 * i, 16), AL] = bot
            a11, a12, a21, a22 = top[:, 0:256], top[:, 256:512], bot[:, 0:256], bot[:, 256:512]
            for q, v in enumerate((a11 + a22, a21 + a22, a11 + a12, a21 - a11, a12 - a22)):
                xa_s[rs(128 * t + 16 * i, 16), tl(2 * q, 2)] = v

    def bcomb(c, src, dst, kw, n1, dcol, srow):
        for i in range(kw // 8):
            ws = [tie(c, src[rs(srow(h, i), 8), tl(n)], c.tok) for h in range(2) for n in (n1, n1 + 1)]
            q = [_even_odd(w) for w in ws]
            res = []
            for p in range(2):
                b11, b12, b21, b22 = (v[p] for v in q)
                res.append((b11 + b22, b12 - b22, b21 - b11, b11 + b12, b21 + b22))
            pks = [_zip2(res[0][j], res[1][j]) for j in range(5)] + [ws[0], ws[3]]
            for j, pk in enumerate(pks):
                dst[rs(j * kw + 8 * i, 8), tl(dcol)] = pk
            c.tok = res[0][1] + (res[0][0] + pltpu.bitcast(pks[4], f32))

    def wcomb(c, ck):
        for m, src in enumerate((wg_u, wu_u)):
            bcomb(c, src, wt_u, 128, 2 * ck, 2 * ck + m, lambda h, i: 128 * h + 8 * i)
            for i in range(8):
                ws = [tie(c, src[rs(256 + 8 * i, 8), tl(n)], c.tok) for n in (2 * ck, 2 * ck + 1)]
                q = [_even_odd(w) for w in ws]
                c.tok = q[0][0] + q[1][0]
                for j, w in enumerate((_zip2(c.tok, q[0][1] + q[1][1]), ws[0], ws[1])):
                    wt_u[rs(896 + 64 * j + 8 * i, 8), tl(2 * ck + m)] = w

    def wdcomb(c, pr):
        srow = lambda h, i: 128 * (i // 8) + 64 * h + 8 * (i % 8)
        bcomb(c, wd_u, wdt_u, 384, 2 * pr, pr, srow)
        for i in range(48):
            w = tie(c, wd_u[rs(srow(pr, i), 8), tl(4)], c.tok)
            wdt_u[rs(7 * 384 + 8 * i, 8), tl(pr)] = w
            c.tok = pltpu.bitcast(w, f32) + 1.0

    def xe(c, o):
        lo64, slo = sm_v[16:24, :] != 0, sm_v[24:32, :] != 0
        rolled = {}

        def roll4(v):
            if id(v) not in rolled:
                rolled[id(v)] = (v, pltpu.roll(v, 4, 0))
            return rolled[id(v)][1]

        def mix(a, b, g):
            return tuple(jnp.where(slo, u, roll4(v)) if g == 0 else jnp.where(slo, roll4(u), v) for u, v in zip(a, b))

        def tiec(v, tok):
            return tuple(tie(c, u, tok) for u in v)

        l01 = jnp.where(lo64, 1.0, 0.0).astype(f32)
        prep = []
        tok = c.tok
        for h in range(2):
            z = tiec((zw_s[0, rs(8 * o, 8), tl(h)], zw_s[1, rs(8 * o, 8), tl(h)]), tok)
            w = (zw_s[2, rs(8 * o, 8), tl(h)], zw_s[3, rs(8 * o, 8), tl(h)])
            pw = {1: z}
            e = 1
            while e < 512:
                pw[2 * e] = _csq(pw[e])
                e *= 2
                if e == 2:
                    wz = _cmul(w, z)
                if e == 8:
                    wz5 = _cmul(wz, pw[4])
            p772 = _cmul(_cmul(pw[256], pw[4]), pw[512])
            er, ei = pw[128]
            if h == 0:
                one, eb = (jnp.ones((8, 128), f32), jnp.zeros((8, 128), f32)), (er, -ei)
            else:
                one, eb = (1.0 - l01, l01), (jnp.where(lo64, ei, er), jnp.where(lo64, er, -ei))
            prep.append((z, wz, wz5, pw[256], p772, pw[8], one, eb))
            if c.xps:
                tok = p772[0]
        tok = p772[0]
        for g in range(2):
            def put(ref, n, lst, h):
                i = len(lst) - 2
                if i % 2 == 0:
                    b0 = (2 * (o % XR) + g) * 8 * n + 8 * i
                    for q, cb in ([(0, 0), (1, 1)] if h == 0 else [(1, 2)]):
                        ref[rs(b0, 16), tl(cb)] = _cat([lst[i][q], lst[i + 1][q]], 0)

            def xseg(h, tok):
                z, wz, wz5, p256, p772 = prep[h][:5]
                xs = [tiec(mix(wz, wz5, g), tok)]
                a1 = mix(z, z, g)
                a256 = am = None
                for src in (0, 1, 2, 1, 3, 5, 6, 7, 8):
                    if len(xs) == 3:
                        a256 = mix(p256, p256, g)
                    if len(xs) == 6:
                        am = mix(p772, p256, g)
                    xs.append(_cmul(xs[src], a1 if len(xs) < 4 else (am if len(xs) == 8 else a256)))
                    put(xs_s, 10, xs, h)
                return xs[-1][1]

            def eseg(hs, tok):
                es, a8 = {}, {}
                for h in hs:
                    p8, one, eb = prep[h][5:]
                    a8[h] = mix(p8, p8, g)
                    es[h] = [tiec(tuple(jnp.where(slo, u, roll4(v) if g == 0 else v) for u, v in zip(one, eb)), tok)]
                if 1 in hs:
                    ra, rb = a8[1][0] + a8[1][0], a8[1][0] * a8[1][0] + a8[1][1] * a8[1][1]
                for v in range(15):
                    for h in hs:
                        if h == 0 or v == 0:
                            es[h].append(_cmulc(es[h][-1], a8[h]))
                        else:
                            es[h].append((None, ra * es[h][-1][1] - rb * es[h][-2][1]))
                        put(es_s, 16, es[h], h)
                return es[hs[0]][-1][1]

            tok = xseg(0, tok)
            tok = eseg([1], eseg([0], tok)) if (c.xs2 and (2 * o + g) % c.xs2 == 0) else eseg([0, 1], tok)
            tok = xseg(1, tok)
        c.tok = tok

    def c2(c, unit):
        ct, p = divmod(unit, 8)
        ys, gs = {}, {}
        for cl in (0, 2, 1, 3):
            rws = rs(64 * cl + 8 * p, 8)
            pos = cl in (0, 3)

            def kpart(pt, s):
                ht = lambda q: cf(off["T", pt[0]] + 256 * q + 64 * cl + 8 * p, 8)
                kd = lambda q: kd_s[ct, _KD[pt, q] + (p % (16 // pt[0]) if q in range(6) else 0)]
                half = pt[3] - pt[2] == 256
                if s == 0:
                    kv = ht(0) * kd(4) + ht(1) * kd(5)
                    return kv if not half else (kv + ht(2) * kd("b") if pos else kv - ht(2) * kd("b"))
                q = (s - 1) ^ (not pos)
                kv, tv = ht(0) * kd(q) + ht(1) * kd(2 + q), ht(2) * kd("a-b" if half and q else "a+b")
                return kv - tv if s == 1 else kv + tv

            k1, ri = None, {}
            for s in range(3):
                U, K, out = [], [], []
                for i in range(NS):
                    U.append(u_s[ct, 0, i, rws, :] + u_s[ct, 1, i, rws, :] if s == 0 else u_s[ct, s - 1, i, rws, :])
                    ks = [kpart(pt, s) for pt in _PARTS if pt[1] == i]
                    if i < 3:
                        ks.append((kw_s[ct, 0, i, rws, :] + kw_s[ct, 1, i, rws, :]) * (-0.5) if s == 0
                                  else kw_s[ct, s - 1, i, rws, :])
                    K.append(ks[0] if len(ks) == 1 else ks[0] + ks[1])
                    ms = list(range(1, i)) + ([0, i] if i else [0])
                    a = tie(c, k1[i] if s else K[ms[0]] * U[i - ms[0]], c.tok)
                    ms = ms if s else ms[1:]
                    while ms:
                        c.cnt += 1
                        pr = K[ms[0]] * U[i - ms[0]]
                        if (not c.ps or c.cnt % c.ps) and len(ms) > 1 and (c.jit or not (s == 2 and cl == 3)):
                            pr = pr + K[ms[1]] * U[i - ms[1]]
                            ms = ms[1:]
                        ms = ms[1:]
                        a = a + pr
                    c.tok = a
                    out.append(a)
                    if s == 2 and cl >= 2:
                        yr, yi, zr, zi = ys[cl - 2][2][i], ys[cl - 2][1][i], a, ri[1][i]
                        g = (yr + zr, yi - zi, yr - zr, yi + zi)
                        if cl == 2:
                            gs[i] = g
                            c.tok = a if c.jit else g[2]
                        else:
                            e = gs[i]
                            hs = ((e[0] + g[0], e[1] - g[1]), (e[2] - g[3], e[3] - g[2]),
                                  (e[0] - g[0], e[1] + g[1]), (e[2] + g[3], e[3] + g[2]))
                            for q, h in enumerate(hs):
                                y_s[rs(512 * ct + 128 * q + 16 * p, 16), tl(i)] = _cat(h, 0)
                            c.tok = a if c.jit else hs[3][1] + hs[0][0]
                if s == 0:
                    k1 = out
                else:
                    ri[s] = out
            ys[cl] = ri

    def ffn1(t, ck, strassen=True):
        top, bot = rs(RB * t, 128), rs(RB * t + 128, 128)
        if strassen:
            cw = tl(2 * ck, 2)
            sa = lambda q: xa_s[rs(128 * t, 128), tl(2 * q, 2)]
            tb = lambda q: wt_s[rs(256 * q, 256), cw]
            tk, k3a, k3b = (wt_s[rs(1792 + 128 * j, 128), cw] for j in range(3))
            m4 = _dot(xn_s[bot, tl(2, 2)], tb(2))
            m2 = _dot(_cat([sa(1), xn_s[bot, tl(4)]], 1), _cat([tb(5), k3a], 0))
            c21 = m2 + m4
            m5 = _dot(_cat([sa(2), xn_s[top, tl(4)]], 1), _cat([tb(6), k3b], 0))
            m3 = _dot(xn_s[top, tl(0, 2)], tb(1))
            c12 = m3 + m5
            m1 = _dot(sa(0), tb(0))
            m7 = _dot(_cat([sa(4), xn_s[top, tl(4)]], 1), _cat([tb(4), tk], 0))
            m6 = _dot(_cat([sa(3), xn_s[bot, tl(4)]], 1), _cat([tb(3), tk], 0))
            c11, c22 = m7 + (m1 + (m4 - m5)), m6 + (m1 + (m3 - m2))
        else:
            xn = xn_s[rs(RB * t, RB), AL]
            r1 = _dot(xn, _cat([wg_v[:, tl(2 * ck)], wu_v[:, tl(2 * ck)]], 1))
            r2 = _dot(xn, _cat([wg_v[:, tl(2 * ck + 1)], wu_v[:, tl(2 * ck + 1)]], 1))
            c11, c21, c12, c22 = r1[:128], r1[128:], r2[:128], r2[128:]
        h11, h12, h21, h22 = (v[:, :128] * v[:, 128:] for v in (c11, c12, c21, c22))
        for q, v in enumerate((h11, h12, h21, h22, h11 + h22, h21 + h22, h11 + h12, h21 - h11, h12 - h22)):
            ha_s[rs(128 * t, 128), tl(6 * q + ck)] = v
        return c21[0:8, 0:128]

    def ufwd(t):
        for c0, n in ((0, 2), (2, 2), (4, 1)):
            e = _dot(sm_s[64:320, AL], xn_s[rs(RB * t, 128), tl(c0, n)])
            o = _dot(sm_s[320:576, AL], xn_s[rs(RB * t + 128, 128), tl(c0, n)])
            for j in range(n):
                er, ei, or_, oi = e[:128, tl(j)], e[128:, tl(j)], o[:128, tl(j)], o[128:, tl(j)]
                u_s[c0 + j, 0, t, 0:128], u_s[c0 + j, 0, t, 128:256] = er + or_, er - or_
                u_s[c0 + j, 1, t, 0:128], u_s[c0 + j, 1, t, 128:256] = ei + oi, oi - ei
            if c0 == 0:
                yield

    def kmm(o):
        lane = jax.lax.broadcasted_iota(i32, (8, 128), 1)
        sub = jax.lax.broadcasted_iota(i32, (8, 128), 0)
        slo = sub < 4
        res = [_nt(xs_s[rs(80 * q, 80), AL], es_s[rs(128 * q, 128), AL]) for q in (2 * (o % XR), 2 * (o % XR) + 1)]
        dk = (lane - sub) & 3

        def merge(r, vs):
            out = None
            for k in reversed(range(len(vs))):
                src = r[8 * vs[k]:8 * vs[k] + 8, :]
                if k:
                    src = pltpu.roll(src, k, 1)
                out = src if out is None else jnp.where(dk == k, src, out)
            return out

        def derot(x):
            x = jnp.where((sub & 1) == 1, pltpu.roll(x, 127, 1), x)
            return jnp.where((sub & 2) == 2, pltpu.roll(x, 126, 1), x)

        ts = []
        for vs, sh in (([0, 1, 2, 3], 1), ([4, 5, 6, 7], 2), ([8, 9], 2)):
            a, b = merge(res[0], vs), merge(res[1], vs)
            a, b = jnp.where(slo, a, pltpu.roll(b, 4, 0)), pltpu.roll(jnp.where(slo, pltpu.roll(a, 4, 0), b), sh, 1)
            m = (dk & sh) == 0
            ts += [jnp.where(m, a, b), jnp.where(m, b, a)]
        for i in range(5):
            kc_s[i, rs(8 * o, 8), :] = derot(ts[i])

    def kfwd(ct):
        kt = lambda tau: kc_s[tau, tl(ct), :].astype(bf16)
        kv = {}
        for tau, lg in _SEL.items():
            v = _nt(big_s[rs(off["D", tau], off["Dn", tau]), AL], kt(tau))
            kv.update({lag: v[rs(8 * j, 8)] for j, lag in enumerate(lg)})
            r0 = 16 * ((len(lg) + 1) // 2)
            for pt in [p for p in _PARTS if p[0] == {3: 4, 4: 8}.get(tau)]:
                st, w, p0, p1 = pt
                n = 16 // st
                d = [[v[rs(r0 + 8 * (n * q + j), 8)] for j in range(n)] for q in range(4)]
                r0 += 32 * n
                vl, vr = kv[256 * (w - 1) + p0], kv[256 * (w - 1) + p1]
                if 256 * (w - 1) + p0 not in lg:
                    hv = vl * 0.5
                    d[0], d[1] = [x - hv for x in d[0]], [x + hv if p0 else x - hv for x in d[1]]
                d += [[(x + y) * (-0.5) for x, y in zip(d[q], d[q + 1])] for q in (0, 2)]
                for q in range(6):
                    for j in range(n):
                        kd_s[ct, _KD[pt, q] + j] = d[q][j]
                if p1 - p0 == 512:
                    kd_s[ct, _KD[pt, "a+b"]] = vl + vr
                else:
                    a, b = (vr, -vl) if p0 else (vl, vr)
                    kd_s[ct, _KD[pt, "a+b"]], kd_s[ct, _KD[pt, "a-b"]], kd_s[ct, _KD[pt, "b"]] = a + b, a - b, b
        yield
        for cb in range(2):
            od, ev = (_nt(big_s[rs(off["B0", t] + 128 * cb, 128), AL], kt(t)) for t in (0, 1))
            sm, df = ev + od, ev - od
            for cl, (e0, f0) in ((cb, (sm[:64], sm[64:])), (cb + 2, (df[64:], df[:64]))):
                pos, rw = cl in (0, 3), rs(64 * cl, 64)
                v = _nt(big_s[rs(off["B1"] + 128 * cl, 128), AL], kt(2)) + cf(128 * cl, 128) * _cat([kv[256]] * 16, 0)
                e1, f1 = v[:64], v[64:]
                kw_s[ct, 0, 0, rw], kw_s[ct, 1, 0, rw] = (f0, -e0) if pos else (-f0, e0)
                kw_s[ct, 0, 1, rw], kw_s[ct, 1, 1, rw] = (e0 + f1, f0 - e1) if pos else (e0 - f1, f0 + e1)
                kw_s[ct, 0, 2, rw], kw_s[ct, 1, 2, rw] = e1, f1
            yield

    def inv(ct, t):
        y = [_dot(big_s[rs(off["I", q], 64), AL], y_s[rs(512 * ct + 128 * q, 128), tl(t)]) for q in range(4)]
        return _zip2(y[0], y[2]), _zip2(y[1], y[3])

    def finish(ct, t, dt_, db_):
        y = inv(ct, t)
        xs = _even_odd(x_u[rs(128 * t, 128), tl(ct)])
        res = []
        for h, dn in enumerate((dt_, db_)):
            yy = pltpu.bitcast(y[h], bf16).astype(f32)
            xn = xn_s[rs(RB * t + 128 * h, 128), tl(ct)].astype(f32)
            res.append(xs[h] + (xn * coef_s[0:1, tl(ct)] + dn) + yy)
        o_u[rs((ct * L + RB * t) // 2, 128), AL] = _zip2(*res)
        c_out[ct * NS + t].start()

    pend = {}

    def flush(ct, t):
        finish(ct, t, *pend.pop((ct, t)))

    def down4(t):
        dn = _dot(_cat([ha_s[rs(128 * t, 128), 0:1536], ha_s[rs(128 * t, 128), 1536:3072]], 0),
                  _cat([wdt_s[5376:6144, tl(0)], wdt_s[5376:6144, tl(1)]], 0))
        pend[4, t] = (dn[:128], dn[128:])

    def down_pair(pr, t):
        m = {}
        for k, (a, b) in ((1, (4, 0)), (4, (3, 2)), (5, (6, 6)), (7, (8, 4)), (2, (5, 5)), (3, (0, 1)), (6, (7, 3))):
            m[k] = _dot(ha_s[rs(128 * t, 128), tl(6 * a, 6)], wdt_s[rs(768 * b, 768), tl(pr)])
            if k == 2:
                pend[2 * pr, t] = (m[7] + m[1] + m[4] - m[5], m[2] + m[4])
            if k == 6:
                pend[2 * pr + 1, t] = (m[3] + m[5], m[6] + m[1] - m[2] + m[3])
            yield

    pars = (are_h, aim_h, bre_h, bim_h, cre_h, cim_h)
    par = lambda a, n: [(p.at[:, tl(a, n)], par_v.at[i, :, tl(a, n)]) for i, p in enumerate(pars)]
    xr = lambda a, b: [(x_hbm.at[a * RB:b * RB], x_v.at[a * RB:b * RB])]
    wch = lambda a, n: [(h.at[:, tl(2 * a, 2 * n)], v.at[:, tl(2 * a, 2 * n)]) for h, v in ((wg_h, wg_v), (wu_h, wu_v))]
    dum = lambda i: [(sm_h.at[0:8], dum_v.at[8 * i:8 * i + 8])]
    G = [grp(p) for p in (
        xr(0, 1), [(sm_h, sm_v)] + xr(1, 2), wch(0, 1), wch(1, 1) + xr(2, 3),
        wch(2, 1) + xr(3, 4) + par(0, 1) + [(ldt_h, ldt_v), (dsk_h, dsk_v)], par(1, 1) + wch(3, 3),
        par(2, 3) + xr(4, 8), [(big_h, big_v), (wd_h, wd_v)], dum(0), dum(1), dum(2))]
    c_out = grp([(o_s.at[rs(ct * L + RB * t, RB)], o_hbm.at[rs(RB * t, RB), tl(ct)])
                 for ct in range(NCT) for t in range(NS)])

    def wait(cs):
        for cc in cs:
            cc.wait()

    def run_all(gen):
        for _ in gen:
            pass

    def part(c, main=(), km=(), uf=(), kf=(), wc=(), wdc=(), lns=(), a0s=(), xes=(), c2s=(),
             late=None, nw=4, nk=None, xps=1, ps=0, xs2=0, nc=2, jit=0):
        c.xps, c.ps, c.xs2, c.jit = xps, ps, xs2, jit
        for ck in wc:
            wcomb(c, ck)
        for pr in wdc:
            wdcomb(c, pr)
        for o in xes:
            xe(c, o)
        for un in c2s:
            c2(c, un)
        extra = []
        for gen, n in [(ufwd(t), 2) for t in uf] + [(kfwd(ct), 3) for ct in kf]:
            extra += [functools.partial(next, gen, None)] * n
        nm, kms, mt = len(main), list(km), []
        nkk = nk if nk is not None else nm - 1
        for i, fn in enumerate(main):
            if i < nkk:
                for o in kms[i * len(kms) // nkk:(i + 1) * len(kms) // nkk]:
                    kmm(o)
            for fx in extra[i * len(extra) // nm:(i + 1) * len(extra) // nm]:
                fx()
            mt.append(fn())
        if a0s or lns:
            keep = c.tok, c.never
            c.tok, c.never = (None if late is None else mt[late]), sm_v[8:16, :] != 0
            for ct in a0s:
                a0(c, ct, nc)
            toks = [c.xt if a0s else c.tok] * nw
            for q in range(1, nw if toks[0] is not None else 0):
                toks[q] = functools.reduce(lambda a, _: a + 1.0, range(20), toks[q - 1])
            for t in lns:
                ln(c, t, toks)
            c.tok, c.never = keep

    def block(waits, *parts, end=()):
        def run():
            wait(waits)
            c = mk()
            for p in parts:
                part(c, **p)
            wait(end)
        return run

    for g in G:
        for cc in g:
            cc.start()
    flag = jax.lax.fori_loop(0, 3, lambda i, a: a + i, 0)
    wait(G[0])
    ln(mk(False), 0, [None])

    def p1():
        wait(G[1])
        run_all(ufwd(0))
        ln(mk(False), 1, [None])
        run_all(ufwd(1))

    R, P = range, functools.partial
    it = [P(ffn1, t, ck) for t, ck in ([(t, ck) for t in (2, 3) for ck in R(3)] + [(t, ck) for t in R(4) for ck in R(3, 6)]
                                       + [(t, ck) for t in R(4, 8) for ck in R(6)])]
    pl_ = lambda ck: [P(ffn1, 0, ck, False), P(ffn1, 1, ck, False)]
    def dots(pr, t):
        return [P(next, down_pair(pr, t), None)] * 7

    def pairs(pr, now, lag):
        out = []
        fl = lambda ct, t: [P(flush, ct, t)] if ct in now and t >= 0 else []
        for t in R(NS):
            d = dots(pr, t)
            if lag:
                out += d[:1] + fl(2 * pr, t - 1) + d[1:3] + fl(2 * pr + 1, t - 1) + d[3:]
            else:
                out += d[:5] + fl(2 * pr, t) + d[5:] + fl(2 * pr + 1, t)
        if lag:
            out = out[:-2] + fl(2 * pr, NS - 1) + out[-2:] + fl(2 * pr + 1, NS - 1)
        return out

    ymain = pairs(0, (0, 1), cfg("lag", 1))
    zn = ((2, 3), (2,), ())[cfg("zd", 2)]
    zmain = pairs(1, zn, cfg("lag", 1))
    for t in R(NS):
        zmain += [P(down4, t)] + [P(flush, ct, t) for ct in (2, 3) if ct not in zn and t < 6] + [P(flush, 4, t)]
        if t in (3, 4, 5, 6) and cfg("zt", 1):
            zmain += [P(flush, 2 + (t + 1) % 2, 6 + (t - 3) // 2)]
    blocks = [
        p1,
        block(G[2], dict(main=pl_(0), wc=[0])),
        block(G[3], dict(main=pl_(1), wc=[1], lns=[2])),
        block(G[4], dict(main=pl_(2) + it[0:2], uf=[2], wc=[2], a0s=[0], lns=[3])),
        block(G[5], dict(main=it[2:6], uf=[3], wc=[3, 4, 5], xes=R(0, 10), a0s=[1], xps=0)),
        block(G[6], dict(main=it[6:18], km=R(0, 10), xes=R(10, 32), lns=[4, 5, 6, 7], a0s=[2, 3], late=cfg("late5", 5), nk=2,
                         nw=cfg("nw5", 5), xps=cfg("xps5", 0), nc=cfg("nc5", 2))),
        block(G[7], dict(main=it[18:cfg("a6", 25)], km=R(10, 32), uf=R(4, 8), wdc=[0, 1], xes=R(32, 64), xs2=cfg("xs6", 1)),
              dict(main=it[cfg("a6", 25):cfg("b6", 29)], kf=[0, 1], a0s=[4], late=cfg("l6", 2), nc=1)),
        block(G[8], dict(main=it[cfg("b6", 29):cfg("a7", 40)], km=R(32, 64), nk=cfg("nk7", 8), xes=R(64, 80), xs2=cfg("xs7", 2), c2s=R(0, 16), ps=cfg("ps7", 2)),
              dict(main=it[cfg("a7", 40):42], kf=[2, 3])),
        block(G[9], dict(main=ymain[:cfg("yk", 56)], km=R(64, 80), nk=40, c2s=R(16, cfg("zc", 27)), ps=cfg("ps8", 1)), dict(main=ymain[cfg("yk", 56):], kf=[4])),
        block(G[10], dict(main=zmain, c2s=R(cfg("zc", 27), 40), ps=cfg("ps9", 3), jit=1), end=c_out),
    ]
    for i, fn in enumerate(blocks):
        if ONLYB is not None and str(i) not in ONLYB.split(","):
            continue
        with jax.named_scope("blk%02d" % i):
            pl.when(flag > -i)(fn)
    if ONLYB is not None:
        for r in (coef_s, zw_s, xn_u, xa_u, ha_u, wt_u, wdt_u, u_s, xs_u, es_u, kc_s, kw_s, kd_s, y_u, o_s):
            cc = pltpu.make_async_copy(r, r, sems.at[12])
            cc.start()
            cc.wait()


@jax.jit
def pallas_parallel_sum__ssm_conv_s4__glu_gated_bilinear__prompt_kernel(A_u, A_A_re, A_A_im, A_B_re, A_B_im, A_C_re, A_C_im, A_log_dt, A_Dskip, B_x, B_w_gate, B_w_up, B_w_down):
    _, big, small = _consts()
    hbm = pl.BlockSpec(memory_space=pltpu.HBM)
    out = pl.pallas_call(
        _kernel,
        in_specs=[hbm] * 14,
        out_specs=hbm,
        out_shape=jax.ShapeDtypeStruct((L, D), bf16),
        scratch_shapes=[
            pltpu.VMEM((L, D), bf16),
            pltpu.VMEM((6, N, D), bf16),
            pltpu.VMEM((D,), bf16), pltpu.VMEM((D,), bf16),
            pltpu.VMEM((D, F), bf16), pltpu.VMEM((D, F), bf16), pltpu.VMEM((F, D), bf16),
            pltpu.VMEM(big.shape, u32), pltpu.VMEM(small.shape, u32),
            pltpu.VMEM((8, D), f32),
            pltpu.VMEM((4, D, 256), f32),
            pltpu.VMEM((L // 2, D), u32),
            pltpu.VMEM((L // 4, 1280), u32),
            pltpu.VMEM((L // 4, 9 * 768), u32),
            pltpu.VMEM((1088, F), u32),
            pltpu.VMEM((8 * 384, 256), u32),
            pltpu.VMEM((NCT, 2, NS, 256, 128), f32),
            pltpu.VMEM((2 * XR * 40, 384), u32),
            pltpu.VMEM((2 * XR * 64, 384), u32),
            pltpu.VMEM((5, D, 128), f32),
            pltpu.VMEM((NCT, 2, 3, 256, 128), f32),
            pltpu.VMEM((NCT, _KD["n"], 8, 128), f32),
            pltpu.VMEM((NCT * 256, NS * 128), u32),
            pltpu.VMEM((NCT * L, 128), bf16),
            pltpu.VMEM((24, 128), u32),
            pltpu.SemaphoreType.DMA((13 if ONLYB else 12,)),
        ],
        compiler_params=pltpu.CompilerParams(vmem_limit_bytes=120 * 1024 * 1024),
    )(A_u.reshape(L, D), A_A_re.T, A_A_im.T, A_B_re.T, A_B_im.T, A_C_re.T, A_C_im.T, A_log_dt, A_Dskip,
      B_w_gate, B_w_up, B_w_down, jnp.asarray(big), jnp.asarray(small))
    return out.reshape(1, L, D)
```

```python
import functools
import numpy as np
import jax
import jax.numpy as jnp
import jax.experimental.pallas as pl
import jax.experimental.pallas.tpu as pltpu

L, D, N, F = 2048, 640, 192, 1536
RB = 256
NS = L // RB
NCT = D // 128
NCK = 6
XR = 56
f32, bf16, u32, i32 = jnp.float32, jnp.bfloat16, jnp.uint32, jnp.int32

_PARTS = [(4, 2, 256, 512), (4, 3, 0, 512), (4, 4, 0, 256), (8, 4, 256, 512), (8, 5, 0, 512), (8, 6, 0, 512), (8, 7, 0, 512)]
_SEL = {1: [256], 2: [512], 3: [768, 1024], 4: [1280, 1536, 1792, 2048]}
_KD = {}
for _p in _PARTS:
    for _n, _w in [(q, 16 // _p[0]) for q in range(6)] + [("a+b", 1), ("a-b", 1), ("b", 1)]:
        _KD[_p, _n] = _KD.get("n", 0)
        _KD["n"] = _KD.get("n", 0) + _w


def _tile_lags():
    lane = np.arange(128)
    q, k = lane // 4, lane % 4
    j8 = 8 * (q // 2 + 16 * (q % 2))
    t = []
    for a0, a1, sh in (([1, 2, 3, 4], [5, 6, 7, 8], 1), ([258, 260, 516, 772], [262, 264, 520, 776], 2),
                       ([1544, 1800, 0, 0], [1032, 1288, 0, 0], 2)):
        a, b = np.asarray(a0)[k] + j8, np.roll(np.asarray(a1)[k] + j8, sh)
        m = lane % (2 * sh) < sh
        t += [np.where(m, a, b), np.where(m, b, a)]
    return np.stack(t[:5])


def _pack_np(a):
    b = np.asarray(a, np.float32).astype(jnp.bfloat16).view(np.uint16).astype(np.uint32)
    return b[0::2] | (b[1::2] << 16)


@functools.lru_cache(maxsize=None)
def _consts():
    rl = np.arange(L).astype(np.float32).astype(jnp.bfloat16).astype(np.int64)
    lags = _tile_lags()
    where = {int(v): (t, l) for t in range(5) for l, v in enumerate(lags[t])}
    r2 = 2 * np.arange(64)
    th = 2 * np.pi * (np.concatenate([r2, 127 - r2, 255 - r2, 128 + r2]) + 0.5) / 512

    def ef(p):
        re, im = np.cos(th * p).reshape(4, 64), -np.sin(th * p).reshape(4, 64)
        return np.stack([im - re, -(re + im)], axis=1).reshape(512)

    rows, off, hf = [], {}, []

    def add(key, m):
        off[key] = sum(x.shape[0] for x in rows)
        rows.append(m)

    for t in (0, 1):
        add(("B0", t), np.stack([ef(p)[:256] for p in lags[t]], axis=1))
    m = np.zeros((512, 128))
    for p in range(2, 257):
        tt, l = where[int(rl[256 + p])]
        assert tt == 2
        m[:, l] += ef(p) * (0.5 if p == 256 else 1.0)
    add("B1", m)
    assert rl[257] == 256
    hf.append(ef(1))
    for tau, lg in _SEL.items():
        parts = [p for p in _PARTS if p[0] == {3: 4, 4: 8}.get(tau)]
        blk = []
        for st, w, p0, p1 in parts:
            nr = 128 // st
            dm = np.zeros((4 * nr, 128))
            for pc in range(p0, p1 + 1, st):
                lag, odd = 256 * (w - 1) + pc, (pc // st) % 2
                assert all(int(rl[lag + d]) == lag for d in range(odd - st // 2, st // 2 + 1 - odd)
                           if p0 < pc + d < p1 and lag + d < L)
                tt, l = where[lag]
                if tt != tau:
                    assert pc == p0
                    continue
                v = ef(pc) * (0.5 if pc in (p0, p1) else 1.0)
                dm[2 * nr * odd:2 * nr * odd + nr, l] += v[0:nr]
                dm[2 * nr * odd + nr:2 * nr * odd + 2 * nr, l] += v[64:64 + nr]
            blk.append(dm)
        sel = np.zeros((16 * ((len(lg) + 1) // 2), 128))
        for j, lag in enumerate(lg):
            assert where[lag][0] == tau
            sel[8 * j:8 * j + 8, where[lag][1]] = 1.0
        add(("D", tau), np.concatenate([sel] + blk, axis=0))
        off["Dn", tau] = rows[-1].shape[0]
    for st in (4, 8):
        ho = 1 + 2 * sum(np.cos(th * d) for d in range(1, st // 2))
        off["T", st] = sum(x.shape[0] for x in hf)
        hf += [ho + 2 * np.cos(th * (st // 2)), ho * (-1.0) ** ((np.arange(256) % 64) // (128 // st)),
               sum(np.sin(th * d) for d in range(1, st // 2 + 1))]
    pos = np.arange(128)
    tc = th[8 * (pos // 16) + pos % 8]
    for c in range(4):
        a = tc[None, :] * (256 + 4 * np.arange(64) + c)[:, None]
        add(("I", c), np.where(pos[None, :] % 16 < 8, np.cos(a), -np.sin(a)) / 256.0)
    fk = _pack_np(np.concatenate(rows, axis=0))
    off["F32"] = fk.shape[0]
    hf = np.repeat(np.concatenate(hf)[:, None], 128, axis=1).astype(np.float32)
    big = np.concatenate([fk, hf.view(np.uint32)], axis=0)
    fu = []
    for par in range(2):
        a = th[:128, None] * (2 * pos + par)[None, :]
        fu.append(_pack_np(np.concatenate([np.cos(a), -np.sin(a)], axis=0)))
    zero = np.zeros((8, 128), np.uint32)
    small = np.concatenate([zero, zero, np.broadcast_to(np.arange(128) < 64, (8, 128)).astype(np.uint32),
                            np.broadcast_to(np.arange(8)[:, None] < 4, (8, 128)).astype(np.uint32)] + fu + [zero], axis=0)
    return off, big, small


class _Packed:
    def __init__(self, ref):
        self.ref = ref

    def __getitem__(self, idx):
        return pltpu.bitcast(self.ref[idx[0].start // 2:idx[0].stop // 2, idx[1]], bf16)

    def __setitem__(self, idx, v):
        self.ref[idx[0].start // 2:idx[0].stop // 2, idx[1]] = pltpu.bitcast(v.astype(bf16), u32)


class _Words:
    def __init__(self, ref):
        self.ref = ref

    def __getitem__(self, idx):
        return pltpu.bitcast(self.ref[2 * idx[0].start:2 * idx[0].stop, idx[1]], u32)

    def __setitem__(self, idx, v):
        self.ref[2 * idx[0].start:2 * idx[0].stop, idx[1]] = pltpu.bitcast(v, bf16)


class _Ctx:
    pass


def _nt(a, b):
    return jax.lax.dot_general(a, b, (((1,), (1,)), ((), ())), preferred_element_type=f32)


def _dot(a, b):
    return jnp.dot(a, b, preferred_element_type=f32)


def _cat(xs, axis):
    return jnp.concatenate(xs, axis=axis)


def _zip2(a, b):
    return pltpu.pack_elementwise([a, b], packed_dtype=bf16)


def _even_odd(w):
    return pltpu.bitcast(w << 16, f32), pltpu.bitcast(w & jnp.uint32(0xFFFF0000), f32)


def _cis(mag, th):
    kf = jnp.floor(th * (2.0 / np.pi) + 0.5)
    k = kf.astype(i32)
    r = ((th - kf * 1.5703125) - kf * 4.837512969970703125e-4) - kf * 7.54978995489188216e-8
    r = jnp.minimum(jnp.maximum(r, -1.0), 1.0)
    r2 = r * r
    s = r + r * (r2 * (-1.6666654611e-1 + r2 * (8.3321608736e-3 + r2 * -1.9515295891e-4)))
    c = 1.0 + r2 * (-0.5 + r2 * (4.166664568298827e-2 + r2 * (-1.388731625493765e-3 + r2 * 2.443315711809948e-5)))
    swap = (k & 1) == 1
    mb = pltpu.bitcast(mag, i32)
    ms = pltpu.bitcast(mb ^ ((k & 2) << 30), f32)
    mc = pltpu.bitcast(mb ^ (((k + 1) & 2) << 30), f32)
    return mc * jnp.where(swap, s, c), ms * jnp.where(swap, c, s)


def _cmul(a, b):
    return a[0] * b[0] - a[1] * b[1], a[0] * b[1] + a[1] * b[0]


def _cmulc(a, b):
    return a[0] * b[0] + a[1] * b[1], a[1] * b[0] - a[0] * b[1]


def _csq(a):
    return a[0] * a[0] - a[1] * a[1], (a[0] + a[0]) * a[1]


def tl(i, n=1):
    return slice(128 * i, 128 * (i + n))


def rs(a, n):
    return slice(a, a + n)


def _kernel(x_hbm, are_h, aim_h, bre_h, bim_h, cre_h, cim_h, ldt_h, dsk_h, wg_h, wu_h, wd_h,
            big_h, sm_h, o_hbm,
            x_v, par_v, ldt_v, dsk_v, wg_v, wu_v, wd_v, big_v, sm_v, coef_s, zw_s, xn_u, xa_u, ha_u,
            wt_u, wdt_u, u_s, xs_u, es_u, kc_s, kw_s, kd_s, y_u, o_s, dum_v, sems):
    off = _consts()[0]
    xn_s, xa_s, ha_s, wt_s, wdt_s, xs_s, es_s, y_s, big_s, sm_s = [
        _Packed(r) for r in (xn_u, xa_u, ha_u, wt_u, wdt_u, xs_u, es_u, y_u, big_v, sm_v)]
    x_u, wg_u, wu_u, wd_u, o_u = [_Words(r) for r in (x_v, wg_v, wu_v, wd_v, o_s)]
    AL = slice(None)
    nsem = [0]

    def grp(pairs):
        nsem[0] += 1
        return [pltpu.make_async_copy(a, b, sems.at[nsem[0] - 1]) for a, b in pairs]

    def cf(r0, n):
        return pltpu.bitcast(big_v[rs(off["F32"] + r0, n), :], f32)

    def mk(paced=True):
        c = _Ctx()
        c.never = (sm_v[0:8, :] != 0) if paced else None
        c.tok = c.xt = None
        c.cnt = 0
        return c

    def tie(c, v, tok):
        if tok is None or c.never is None:
            return v
        if tok.dtype != v.dtype:
            tok = pltpu.bitcast(tok, v.dtype)
        h = jnp.where(c.never, tok, v[:, :128])
        return h if v.shape[1] == 128 else _cat([h, v[:, 128:]], 1)

    def a0(c, ct, nc):
        cs = tl(ct)
        dt = jnp.exp(ldt_v[...].astype(f32).reshape(1, D)[:, cs]).astype(bf16).astype(f32)
        outs = [[], [], [], []]
        k0 = None
        toks = [c.tok] * nc
        for i in range(N // 8):
            ld = lambda q: par_v[q, 8 * i:8 * i + 8, cs].astype(f32)
            tk = toks[i % nc]
            zr, zi = _cis(jnp.exp(dt * ld(0)), tie(c, dt * ld(1), tk))
            cb = _cmul((ld(4), ld(5)), (tie(c, ld(2), tk), tie(c, ld(3), tk)))
            wr, wi = dt * cb[0], dt * cb[1]
            k0 = wr if k0 is None else k0 + wr
            toks[i % nc] = zr
            for o, v in zip(outs, (zr, zi, wr, wi)):
                o.append(v)
        c.tok = toks[-1]
        coef_s[:, cs] = jnp.broadcast_to(
            jnp.sum(k0, axis=0, keepdims=True) + dsk_v[...].astype(f32).reshape(1, D)[:, cs], (8, 128))
        hi = [outs[0][16:] * 2, outs[1][16:] * 2, [-v for v in outs[3][16:]] + outs[2][16:], outs[2][16:] + outs[3][16:]]
        for q in range(4):
            for h, v in enumerate((_cat(outs[q][:16], 0).T, _cat(hi[q], 0).T)):
                zw_s[q, cs, tl(h)] = v
                c.xt = v[120:128] if c.xt is None else c.xt + v[120:128]

    def ln(c, t, toks):
        for i in range(8):
            eo = ([], [])
            for g in range(2):
                wr = rs(128 * t + 16 * i + 8 * g, 8)
                for hh, xx in enumerate(_even_odd(x_u[wr, AL])):
                    ci = (4 * i + 2 * g + hh) % len(toks)
                    xx = tie(c, xx, toks[ci])
                    mu = jnp.sum(xx, axis=1, keepdims=True) * (1.0 / D)
                    var = jnp.maximum(jnp.sum(xx * xx, axis=1, keepdims=True) * (1.0 / D) - mu * mu, 0.0)
                    if c.never is not None:
                        xx = pltpu.unpack_elementwise(x_u[wr, AL], index=hh, packed_dtype=bf16, unpacked_dtype=f32)
                    xn = (xx - mu) * jax.lax.rsqrt(var + 1e-5)
                    toks[ci] = xn[:, :128]
                    eo[hh].append(xn)
            top, bot = _cat(eo[0], 0), _cat(eo[1], 0)
            xn_s[rs(RB * t + 16 * i, 16), AL] = top
            xn_s[rs(RB * t + 128 + 16 * i, 16), AL] = bot
            a11, a12, a21, a22 = top[:, 0:256], top[:, 256:512], bot[:, 0:256], bot[:, 256:512]
            for q, v in enumerate((a11 + a22, a21 + a22, a11 + a12, a21 - a11, a12 - a22)):
                xa_s[rs(128 * t + 16 * i, 16), tl(2 * q, 2)] = v

    def bcomb(c, src, dst, kw, n1, dcol, srow):
        for i in range(kw // 8):
            ws = [tie(c, src[rs(srow(h, i), 8), tl(n)], c.tok) for h in range(2) for n in (n1, n1 + 1)]
            q = [_even_odd(w) for w in ws]
            res = []
            for p in range(2):
                b11, b12, b21, b22 = (v[p] for v in q)
                res.append((b11 + b22, b12 - b22, b21 - b11, b11 + b12, b21 + b22))
            pks = [_zip2(res[0][j], res[1][j]) for j in range(5)] + [ws[0], ws[3]]
            for j, pk in enumerate(pks):
                dst[rs(j * kw + 8 * i, 8), tl(dcol)] = pk
            c.tok = res[0][1] + (res[0][0] + pltpu.bitcast(pks[4], f32))

    def wcomb(c, ck):
        for m, src in enumerate((wg_u, wu_u)):
            bcomb(c, src, wt_u, 128, 2 * ck, 2 * ck + m, lambda h, i: 128 * h + 8 * i)
            for i in range(8):
                ws = [tie(c, src[rs(256 + 8 * i, 8), tl(n)], c.tok) for n in (2 * ck, 2 * ck + 1)]
                q = [_even_odd(w) for w in ws]
                c.tok = q[0][0] + q[1][0]
                for j, w in enumerate((_zip2(c.tok, q[0][1] + q[1][1]), ws[0], ws[1])):
                    wt_u[rs(896 + 64 * j + 8 * i, 8), tl(2 * ck + m)] = w

    def wdcomb(c, pr):
        srow = lambda h, i: 128 * (i // 8) + 64 * h + 8 * (i % 8)
        bcomb(c, wd_u, wdt_u, 384, 2 * pr, pr, srow)
        for i in range(48):
            w = tie(c, wd_u[rs(srow(pr, i), 8), tl(4)], c.tok)
            wdt_u[rs(7 * 384 + 8 * i, 8), tl(pr)] = w
            c.tok = pltpu.bitcast(w, f32) + 1.0

    def xe(c, o):
        lo64, slo = sm_v[16:24, :] != 0, sm_v[24:32, :] != 0
        rolled = {}

        def roll4(v):
            if id(v) not in rolled:
                rolled[id(v)] = (v, pltpu.roll(v, 4, 0))
            return rolled[id(v)][1]

        def mix(a, b, g):
            return tuple(jnp.where(slo, u, roll4(v)) if g == 0 else jnp.where(slo, roll4(u), v) for u, v in zip(a, b))

        def tiec(v, tok):
            return tuple(tie(c, u, tok) for u in v)

        l01 = jnp.where(lo64, 1.0, 0.0).astype(f32)
        prep = []
        tok = c.tok
        for h in range(2):
            z = tiec((zw_s[0, rs(8 * o, 8), tl(h)], zw_s[1, rs(8 * o, 8), tl(h)]), tok)
            w = (zw_s[2, rs(8 * o, 8), tl(h)], zw_s[3, rs(8 * o, 8), tl(h)])
            pw = {1: z}
            e = 1
            while e < 512:
                pw[2 * e] = _csq(pw[e])
                e *= 2
                if e == 2:
                    wz = _cmul(w, z)
                if e == 8:
                    wz5 = _cmul(wz, pw[4])
            p772 = _cmul(_cmul(pw[256], pw[4]), pw[512])
            er, ei = pw[128]
            if h == 0:
                one, eb = (jnp.ones((8, 128), f32), jnp.zeros((8, 128), f32)), (er, -ei)
            else:
                one, eb = (1.0 - l01, l01), (jnp.where(lo64, ei, er), jnp.where(lo64, er, -ei))
            prep.append((z, wz, wz5, pw[256], p772, pw[8], one, eb))
            if c.xps:
                tok = p772[0]
        tok = p772[0]
        for g in range(2):
            def put(ref, n, lst, h):
                i = len(lst) - 2
                if i % 2 == 0:
                    b0 = (2 * (o % XR) + g) * 8 * n + 8 * i
                    for q, cb in ([(0, 0), (1, 1)] if h == 0 else [(1, 2)]):
                        ref[rs(b0, 16), tl(cb)] = _cat([lst[i][q], lst[i + 1][q]], 0)

            def xseg(h, tok):
                z, wz, wz5, p256, p772 = prep[h][:5]
                xs = [tiec(mix(wz, wz5, g), tok)]
                a1 = mix(z, z, g)
                a256 = am = None
                for src in (0, 1, 2, 1, 3, 5, 6, 7, 8):
                    if len(xs) == 3:
                        a256 = mix(p256, p256, g)
                    if len(xs) == 6:
                        am = mix(p772, p256, g)
                    xs.append(_cmul(xs[src], a1 if len(xs) < 4 else (am if len(xs) == 8 else a256)))
                    put(xs_s, 10, xs, h)
                return xs[-1][1]

            def eseg(hs, tok):
                es, a8 = {}, {}
                for h in hs:
                    p8, one, eb = prep[h][5:]
                    a8[h] = mix(p8, p8, g)
                    es[h] = [tiec(tuple(jnp.where(slo, u, roll4(v) if g == 0 else v) for u, v in zip(one, eb)), tok)]
                if 1 in hs:
                    ra, rb = a8[1][0] + a8[1][0], a8[1][0] * a8[1][0] + a8[1][1] * a8[1][1]
                for v in range(15):
                    for h in hs:
                        if h == 0 or v == 0:
                            es[h].append(_cmulc(es[h][-1], a8[h]))
                        else:
                            es[h].append((None, ra * es[h][-1][1] - rb * es[h][-2][1]))
                        put(es_s, 16, es[h], h)
                return es[hs[0]][-1][1]

            tok = xseg(0, tok)
            tok = eseg([1], eseg([0], tok)) if (c.xs2 and (2 * o + g) % c.xs2 == 0) else eseg([0, 1], tok)
            tok = xseg(1, tok)
        c.tok = tok

    def c2(c, unit):
        ct, p = divmod(unit, 8)
        ys, gs = {}, {}
        for cl in (0, 2, 1, 3):
            rws = rs(64 * cl + 8 * p, 8)
            pos = cl in (0, 3)

            def kpart(pt, s):
                ht = lambda q: cf(off["T", pt[0]] + 256 * q + 64 * cl + 8 * p, 8)
                kd = lambda q: kd_s[ct, _KD[pt, q] + (p % (16 // pt[0]) if q in range(6) else 0)]
                half = pt[3] - pt[2] == 256
                if s == 0:
                    kv = ht(0) * kd(4) + ht(1) * kd(5)
                    return kv if not half else (kv + ht(2) * kd("b") if pos else kv - ht(2) * kd("b"))
                q = (s - 1) ^ (not pos)
                kv, tv = ht(0) * kd(q) + ht(1) * kd(2 + q), ht(2) * kd("a-b" if half and q else "a+b")
                return kv - tv if s == 1 else kv + tv

            k1, ri = None, {}
            for s in range(3):
                U, K, out = [], [], []
                for i in range(NS):
                    U.append(u_s[ct, 0, i, rws, :] + u_s[ct, 1, i, rws, :] if s == 0 else u_s[ct, s - 1, i, rws, :])
                    ks = [kpart(pt, s) for pt in _PARTS if pt[1] == i]
                    if i < 3:
                        ks.append((kw_s[ct, 0, i, rws, :] + kw_s[ct, 1, i, rws, :]) * (-0.5) if s == 0
                                  else kw_s[ct, s - 1, i, rws, :])
                    K.append(ks[0] if len(ks) == 1 else ks[0] + ks[1])
                    ms = list(range(1, i)) + ([0, i] if i else [0])
                    a = tie(c, k1[i] if s else K[ms[0]] * U[i - ms[0]], c.tok)
                    ms = ms if s else ms[1:]
                    while ms:
                        c.cnt += 1
                        pr = K[ms[0]] * U[i - ms[0]]
                        if (not c.ps or c.cnt % c.ps) and len(ms) > 1 and (c.jit or not (s == 2 and cl == 3)):
                            pr = pr + K[ms[1]] * U[i - ms[1]]
                            ms = ms[1:]
                        ms = ms[1:]
                        a = a + pr
                    c.tok = a
                    out.append(a)
                    if s == 2 and cl >= 2:
                        yr, yi, zr, zi = ys[cl - 2][2][i], ys[cl - 2][1][i], a, ri[1][i]
                        g = (yr + zr, yi - zi, yr - zr, yi + zi)
                        if cl == 2:
                            gs[i] = g
                            c.tok = a if c.jit else g[2]
                        else:
                            e = gs[i]
                            hs = ((e[0] + g[0], e[1] - g[1]), (e[2] - g[3], e[3] - g[2]),
                                  (e[0] - g[0], e[1] + g[1]), (e[2] + g[3], e[3] + g[2]))
                            for q, h in enumerate(hs):
                                y_s[rs(512 * ct + 128 * q + 16 * p, 16), tl(i)] = _cat(h, 0)
                            c.tok = a if c.jit else hs[3][1] + hs[0][0]
                if s == 0:
                    k1 = out
                else:
                    ri[s] = out
            ys[cl] = ri

    def ffn1(t, ck, strassen=True):
        top, bot = rs(RB * t, 128), rs(RB * t + 128, 128)
        if strassen:
            cw = tl(2 * ck, 2)
            sa = lambda q: xa_s[rs(128 * t, 128), tl(2 * q, 2)]
            tb = lambda q: wt_s[rs(256 * q, 256), cw]
            tk, k3a, k3b = (wt_s[rs(1792 + 128 * j, 128), cw] for j in range(3))
            m4 = _dot(xn_s[bot, tl(2, 2)], tb(2))
            m2 = _dot(_cat([sa(1), xn_s[bot, tl(4)]], 1), _cat([tb(5), k3a], 0))
            c21 = m2 + m4
            m5 = _dot(_cat([sa(2), xn_s[top, tl(4)]], 1), _cat([tb(6), k3b], 0))
            m3 = _dot(xn_s[top, tl(0, 2)], tb(1))
            c12 = m3 + m5
            m1 = _dot(sa(0), tb(0))
            m7 = _dot(_cat([sa(4), xn_s[top, tl(4)]], 1), _cat([tb(4), tk], 0))
            m6 = _dot(_cat([sa(3), xn_s[bot, tl(4)]], 1), _cat([tb(3), tk], 0))
            c11, c22 = m7 + (m1 + (m4 - m5)), m6 + (m1 + (m3 - m2))
        else:
            xn = xn_s[rs(RB * t, RB), AL]
            r1 = _dot(xn, _cat([wg_v[:, tl(2 * ck)], wu_v[:, tl(2 * ck)]], 1))
            r2 = _dot(xn, _cat([wg_v[:, tl(2 * ck + 1)], wu_v[:, tl(2 * ck + 1)]], 1))
            c11, c21, c12, c22 = r1[:128], r1[128:], r2[:128], r2[128:]
        h11, h12, h21, h22 = (v[:, :128] * v[:, 128:] for v in (c11, c12, c21, c22))
        for q, v in enumerate((h11, h12, h21, h22, h11 + h22, h21 + h22, h11 + h12, h21 - h11, h12 - h22)):
            ha_s[rs(128 * t, 128), tl(6 * q + ck)] = v
        return c21[0:8, 0:128]

    def ufwd(t):
        for c0, n in ((0, 2), (2, 2), (4, 1)):
            e = _dot(sm_s[64:320, AL], xn_s[rs(RB * t, 128), tl(c0, n)])
            o = _dot(sm_s[320:576, AL], xn_s[rs(RB * t + 128, 128), tl(c0, n)])
            for j in range(n):
                er, ei, or_, oi = e[:128, tl(j)], e[128:, tl(j)], o[:128, tl(j)], o[128:, tl(j)]
                u_s[c0 + j, 0, t, 0:128], u_s[c0 + j, 0, t, 128:256] = er + or_, er - or_
                u_s[c0 + j, 1, t, 0:128], u_s[c0 + j, 1, t, 128:256] = ei + oi, oi - ei
            if c0 == 0:
                yield

    def kmm(o):
        lane = jax.lax.broadcasted_iota(i32, (8, 128), 1)
        sub = jax.lax.broadcasted_iota(i32, (8, 128), 0)
        slo = sub < 4
        res = [_nt(xs_s[rs(80 * q, 80), AL], es_s[rs(128 * q, 128), AL]) for q in (2 * (o % XR), 2 * (o % XR) + 1)]
        dk = (lane - sub) & 3

        def merge(r, vs):
            out = None
            for k in reversed(range(len(vs))):
                src = r[8 * vs[k]:8 * vs[k] + 8, :]
                if k:
                    src = pltpu.roll(src, k, 1)
                out = src if out is None else jnp.where(dk == k, src, out)
            return out

        def derot(x):
            x = jnp.where((sub & 1) == 1, pltpu.roll(x, 127, 1), x)
            return jnp.where((sub & 2) == 2, pltpu.roll(x, 126, 1), x)

        ts = []
        for vs, sh in (([0, 1, 2, 3], 1), ([4, 5, 6, 7], 2), ([8, 9], 2)):
            a, b = merge(res[0], vs), merge(res[1], vs)
            a, b = jnp.where(slo, a, pltpu.roll(b, 4, 0)), pltpu.roll(jnp.where(slo, pltpu.roll(a, 4, 0), b), sh, 1)
            m = (dk & sh) == 0
            ts += [jnp.where(m, a, b), jnp.where(m, b, a)]
        for i in range(5):
            kc_s[i, rs(8 * o, 8), :] = derot(ts[i])

    def kfwd(ct):
        kt = lambda tau: kc_s[tau, tl(ct), :].astype(bf16)
        kv = {}
        for tau, lg in _SEL.items():
            v = _nt(big_s[rs(off["D", tau], off["Dn", tau]), AL], kt(tau))
            kv.update({lag: v[rs(8 * j, 8)] for j, lag in enumerate(lg)})
            r0 = 16 * ((len(lg) + 1) // 2)
            for pt in [p for p in _PARTS if p[0] == {3: 4, 4: 8}.get(tau)]:
                st, w, p0, p1 = pt
                n = 16 // st
                d = [[v[rs(r0 + 8 * (n * q + j), 8)] for j in range(n)] for q in range(4)]
                r0 += 32 * n
                vl, vr = kv[256 * (w - 1) + p0], kv[256 * (w - 1) + p1]
                if 256 * (w - 1) + p0 not in lg:
                    hv = vl * 0.5
                    d[0], d[1] = [x - hv for x in d[0]], [x + hv if p0 else x - hv for x in d[1]]
                d += [[(x + y) * (-0.5) for x, y in zip(d[q], d[q + 1])] for q in (0, 2)]
                for q in range(6):
                    for j in range(n):
                        kd_s[ct, _KD[pt, q] + j] = d[q][j]
                if p1 - p0 == 512:
                    kd_s[ct, _KD[pt, "a+b"]] = vl + vr
                else:
                    a, b = (vr, -vl) if p0 else (vl, vr)
                    kd_s[ct, _KD[pt, "a+b"]], kd_s[ct, _KD[pt, "a-b"]], kd_s[ct, _KD[pt, "b"]] = a + b, a - b, b
        yield
        for cb in range(2):
            od, ev = (_nt(big_s[rs(off["B0", t] + 128 * cb, 128), AL], kt(t)) for t in (0, 1))
            sm, df = ev + od, ev - od
            for cl, (e0, f0) in ((cb, (sm[:64], sm[64:])), (cb + 2, (df[64:], df[:64]))):
                pos, rw = cl in (0, 3), rs(64 * cl, 64)
                v = _nt(big_s[rs(off["B1"] + 128 * cl, 128), AL], kt(2)) + cf(128 * cl, 128) * _cat([kv[256]] * 16, 0)
                e1, f1 = v[:64], v[64:]
                kw_s[ct, 0, 0, rw], kw_s[ct, 1, 0, rw] = (f0, -e0) if pos else (-f0, e0)
                kw_s[ct, 0, 1, rw], kw_s[ct, 1, 1, rw] = (e0 + f1, f0 - e1) if pos else (e0 - f1, f0 + e1)
                kw_s[ct, 0, 2, rw], kw_s[ct, 1, 2, rw] = e1, f1
            yield

    def inv(ct, t):
        y = [_dot(big_s[rs(off["I", q], 64), AL], y_s[rs(512 * ct + 128 * q, 128), tl(t)]) for q in range(4)]
        return _zip2(y[0], y[2]), _zip2(y[1], y[3])

    def finish(ct, t, dt_, db_):
        y = inv(ct, t)
        xs = _even_odd(x_u[rs(128 * t, 128), tl(ct)])
        res = []
        for h, dn in enumerate((dt_, db_)):
            yy = pltpu.bitcast(y[h], bf16).astype(f32)
            xn = xn_s[rs(RB * t + 128 * h, 128), tl(ct)].astype(f32)
            res.append(xs[h] + (xn * coef_s[0:1, tl(ct)] + dn) + yy)
        o_u[rs((ct * L + RB * t) // 2, 128), AL] = _zip2(*res)
        c_out[ct * NS + t].start()

    pend = {}

    def flush(ct, t):
        finish(ct, t, *pend.pop((ct, t)))

    def down4(t):
        dn = _dot(_cat([ha_s[rs(128 * t, 128), 0:1536], ha_s[rs(128 * t, 128), 1536:3072]], 0),
                  _cat([wdt_s[5376:6144, tl(0)], wdt_s[5376:6144, tl(1)]], 0))
        pend[4, t] = (dn[:128], dn[128:])

    def down_pair(pr, t):
        m = {}
        for k, (a, b) in ((1, (4, 0)), (4, (3, 2)), (5, (6, 6)), (7, (8, 4)), (2, (5, 5)), (3, (0, 1)), (6, (7, 3))):
            m[k] = _dot(ha_s[rs(128 * t, 128), tl(6 * a, 6)], wdt_s[rs(768 * b, 768), tl(pr)])
            if k == 2:
                pend[2 * pr, t] = (m[7] + m[1] + m[4] - m[5], m[2] + m[4])
            if k == 6:
                pend[2 * pr + 1, t] = (m[3] + m[5], m[6] + m[1] - m[2] + m[3])
            yield

    pars = (are_h, aim_h, bre_h, bim_h, cre_h, cim_h)
    par = lambda a, n: [(p.at[:, tl(a, n)], par_v.at[i, :, tl(a, n)]) for i, p in enumerate(pars)]
    xr = lambda a, b: [(x_hbm.at[a * RB:b * RB], x_v.at[a * RB:b * RB])]
    wch = lambda a, n: [(h.at[:, tl(2 * a, 2 * n)], v.at[:, tl(2 * a, 2 * n)]) for h, v in ((wg_h, wg_v), (wu_h, wu_v))]
    dum = lambda i: [(sm_h.at[0:8], dum_v.at[8 * i:8 * i + 8])]
    G = [grp(p) for p in (
        xr(0, 1), [(sm_h, sm_v)] + xr(1, 2), wch(0, 1), wch(1, 1) + xr(2, 3),
        wch(2, 1) + xr(3, 4) + par(0, 1) + [(ldt_h, ldt_v), (dsk_h, dsk_v)], par(1, 1) + wch(3, 3),
        par(2, 3) + xr(4, 8), [(big_h, big_v), (wd_h, wd_v)], dum(0), dum(1), dum(2))]
    c_out = grp([(o_s.at[rs(ct * L + RB * t, RB)], o_hbm.at[rs(RB * t, RB), tl(ct)])
                 for ct in range(NCT) for t in range(NS)])

    def wait(cs):
        for cc in cs:
            cc.wait()

    def run_all(gen):
        for _ in gen:
            pass

    def part(c, main=(), km=(), uf=(), kf=(), wc=(), wdc=(), lns=(), a0s=(), xes=(), c2s=(),
             late=None, nw=4, nk=None, xps=1, ps=0, xs2=0, nc=2, jit=0, wcj=()):
        c.xps, c.ps, c.xs2, c.jit = xps, ps, xs2, jit
        if wcj:
            keep = c.tok, c.never
            c.tok, c.never = None, sm_v[288:296, :] != 0
            for ck in wcj:
                wcomb(c, ck)
            c.tok, c.never = keep
        for ck in wc:
            wcomb(c, ck)
        for pr in wdc:
            wdcomb(c, pr)
        for o in xes:
            xe(c, o)
        for un in c2s:
            c2(c, un)
        extra = []
        for gen, n in [(ufwd(t), 2) for t in uf] + [(kfwd(ct), 3) for ct in kf]:
            extra += [functools.partial(next, gen, None)] * n
        nm, kms, mt = len(main), list(km), []
        nkk = nk if nk is not None else nm - 1
        for i, fn in enumerate(main):
            if i < nkk:
                for o in kms[i * len(kms) // nkk:(i + 1) * len(kms) // nkk]:
                    kmm(o)
            for fx in extra[i * len(extra) // nm:(i + 1) * len(extra) // nm]:
                fx()
            mt.append(fn())
        if a0s or lns:
            keep = c.tok, c.never
            c.tok, c.never = (None if late is None else mt[late]), sm_v[8:16, :] != 0
            for ct in a0s:
                a0(c, ct, nc)
            toks = [c.xt if a0s else c.tok] * nw
            for q in range(1, nw if toks[0] is not None else 0):
                toks[q] = functools.reduce(lambda a, _: a + 1.0, range(20), toks[q - 1])
            for t in lns:
                ln(c, t, toks)
            c.tok, c.never = keep

    def block(waits, *parts, end=()):
        def run():
            wait(waits)
            c = mk()
            for p in (parts[0]() if callable(parts[0]) else parts):
                part(c, **p)
            wait(end)
        return run

    for g in G:
        for cc in g:
            cc.start()
    flag = jax.lax.fori_loop(0, 3, lambda i, a: a + i, 0)
    wait(G[0])
    ln(mk(False), 0, [None])

    def p1():
        wait(G[1])
        run_all(ufwd(0))
        ln(mk(False), 1, [None])
        run_all(ufwd(1))

    R, P = range, functools.partial
    it = [P(ffn1, t, ck) for t, ck in ([(t, ck) for t in (2, 3) for ck in R(3)] + [(t, ck) for t in R(4) for ck in R(3, 6)]
                                       + [(t, ck) for t in R(4, 8) for ck in R(6)])]

    def pairs(pr, inline):
        out = []
        fl = lambda ct, t: [P(flush, ct, t)] if inline and t >= 0 else []
        for t in R(NS):
            d = [P(next, down_pair(pr, t), None)] * 7
            out += d[:1] + fl(2 * pr, t - 1) + d[1:3] + fl(2 * pr + 1, t - 1) + d[3:]
        return out[:-2] + fl(2 * pr, NS - 1) + out[-2:] + fl(2 * pr + 1, NS - 1)

    def yparts():
        m = pairs(0, True)
        return [dict(main=m[:56], km=R(64, 80), nk=40, c2s=R(16, 27), ps=1),
                dict(main=m[56:], kf=[4])]

    def zparts():
        m = pairs(1, False)
        for t in R(NS):
            m += [P(down4, t)] + [P(flush, ct, t) for ct in (2, 3) if t < 6] + [P(flush, 4, t)]
            if 3 <= t <= 6:
                m += [P(flush, 2 + (t + 1) % 2, 6 + (t - 3) // 2)]
        return [dict(main=m, c2s=R(27, 40), ps=3, jit=1)]

    blocks = [
        p1,
        block(G[2], dict(main=[P(ffn1, 0, 0, False), P(ffn1, 1, 0)], wcj=[0])),
        block(G[3], dict(main=[P(ffn1, 0, 1, False), P(ffn1, 1, 1)], wcj=[1], lns=[2])),
        block(G[4], dict(main=it[0:2] + [P(ffn1, 0, 2), P(ffn1, 1, 2)], uf=[2], wcj=[2], a0s=[0], lns=[3])),
        block(G[5], dict(main=it[2:6], uf=[3], wc=[3, 4, 5], xes=R(0, 10), a0s=[1], xps=0)),
        block(G[6], dict(main=it[6:18], km=R(0, 10), xes=R(10, 32), lns=[4, 5, 6, 7], a0s=[2, 3], late=5, nk=2,
                         nw=5, xps=0, nc=2)),
        block(G[7], dict(main=it[18:25], km=R(10, 32), uf=R(4, 8), wdc=[0, 1], xes=R(32, 64), xs2=1),
              dict(main=it[25:29], kf=[0, 1], a0s=[4], late=2, nc=1)),
        block(G[8], dict(main=it[29:40], km=R(32, 64), nk=8, xes=R(64, 80), xs2=2, c2s=R(0, 16), ps=2),
              dict(main=it[40:42], kf=[2, 3])),
        block(G[9], yparts),
        block(G[10], zparts, end=c_out),
    ]
    for i, fn in enumerate(blocks):
        pl.when(flag > -i)(fn)


@jax.jit
def pallas_parallel_sum__ssm_conv_s4__glu_gated_bilinear__prompt_kernel(A_u, A_A_re, A_A_im, A_B_re, A_B_im, A_C_re, A_C_im, A_log_dt, A_Dskip, B_x, B_w_gate, B_w_up, B_w_down):
    _, big, small = _consts()
    hbm = pl.BlockSpec(memory_space=pltpu.HBM)
    out = pl.pallas_call(
        _kernel,
        in_specs=[hbm] * 14,
        out_specs=hbm,
        out_shape=jax.ShapeDtypeStruct((L, D), bf16),
        scratch_shapes=[
            pltpu.VMEM((L, D), bf16),
            pltpu.VMEM((6, N, D), bf16),
            pltpu.VMEM((D,), bf16), pltpu.VMEM((D,), bf16),
            pltpu.VMEM((D, F), bf16), pltpu.VMEM((D, F), bf16), pltpu.VMEM((F, D), bf16),
            pltpu.VMEM(big.shape, u32), pltpu.VMEM(small.shape, u32),
            pltpu.VMEM((8, D), f32),
            pltpu.VMEM((4, D, 256), f32),
            pltpu.VMEM((L // 2, D), u32),
            pltpu.VMEM((L // 4, 1280), u32),
            pltpu.VMEM((L // 4, 9 * 768), u32),
            pltpu.VMEM((1088, F), u32),
            pltpu.VMEM((8 * 384, 256), u32),
            pltpu.VMEM((NCT, 2, NS, 256, 128), f32),
            pltpu.VMEM((2 * XR * 40, 384), u32),
            pltpu.VMEM((2 * XR * 64, 384), u32),
            pltpu.VMEM((5, D, 128), f32),
            pltpu.VMEM((NCT, 2, 3, 256, 128), f32),
            pltpu.VMEM((NCT, _KD["n"], 8, 128), f32),
            pltpu.VMEM((NCT * 256, NS * 128), u32),
            pltpu.VMEM((NCT * L, 128), bf16),
            pltpu.VMEM((24, 128), u32),
            pltpu.SemaphoreType.DMA((12,)),
        ],
        compiler_params=pltpu.CompilerParams(vmem_limit_bytes=110 * 1024 * 1024),
    )(A_u.reshape(L, D), A_A_re.T, A_A_im.T, A_B_re.T, A_B_im.T, A_C_re.T, A_C_im.T, A_log_dt, A_Dskip,
      B_w_gate, B_w_up, B_w_down, jnp.asarray(big), jnp.asarray(small))
    return out.reshape(1, L, D)
```

```python
import functools
import numpy as np
import jax
import jax.numpy as jnp
import jax.experimental.pallas as pl
import jax.experimental.pallas.tpu as pltpu

L, D, N, F = 2048, 640, 192, 1536
RB = 256
NS = L // RB
NCT = D // 128
NCK = 6
XR = 56
f32, bf16, u32, i32 = jnp.float32, jnp.bfloat16, jnp.uint32, jnp.int32

_PARTS = [(4, 2, 256, 512), (4, 3, 0, 512), (4, 4, 0, 256), (8, 4, 256, 512), (8, 5, 0, 512), (8, 6, 0, 512), (8, 7, 0, 512)]
_SEL = {1: [256], 2: [512], 3: [768, 1024], 4: [1280, 1536, 1792, 2048]}
_KD = {}
for _p in _PARTS:
    for _n, _w in [(q, 16 // _p[0]) for q in range(6)] + [("a+b", 1), ("a-b", 1), ("b", 1)]:
        _KD[_p, _n] = _KD.get("n", 0)
        _KD["n"] = _KD.get("n", 0) + _w


def _tile_lags():
    lane = np.arange(128)
    q, k = lane // 4, lane % 4
    j8 = 8 * (q // 2 + 16 * (q % 2))
    t = []
    for a0, a1, sh in (([1, 2, 3, 4], [5, 6, 7, 8], 1), ([258, 260, 516, 772], [262, 264, 520, 776], 2),
                       ([1544, 1800, 0, 0], [1032, 1288, 0, 0], 2)):
        a, b = np.asarray(a0)[k] + j8, np.roll(np.asarray(a1)[k] + j8, sh)
        m = lane % (2 * sh) < sh
        t += [np.where(m, a, b), np.where(m, b, a)]
    return np.stack(t[:5])


def _pack_np(a):
    b = np.asarray(a, np.float32).astype(jnp.bfloat16).view(np.uint16).astype(np.uint32)
    return b[0::2] | (b[1::2] << 16)


@functools.lru_cache(maxsize=None)
def _consts():
    rl = np.arange(L).astype(np.float32).astype(jnp.bfloat16).astype(np.int64)
    lags = _tile_lags()
    where = {int(v): (t, l) for t in range(5) for l, v in enumerate(lags[t])}
    r2 = 2 * np.arange(64)
    th = 2 * np.pi * (np.concatenate([r2, 127 - r2, 255 - r2, 128 + r2]) + 0.5) / 512

    def ef(p):
        re, im = np.cos(th * p).reshape(4, 64), -np.sin(th * p).reshape(4, 64)
        return np.stack([im - re, -(re + im)], axis=1).reshape(512)

    rows, off, hf = [], {}, []

    def add(key, m):
        off[key] = sum(x.shape[0] for x in rows)
        rows.append(m)

    for t in (0, 1):
        add(("B0", t), np.stack([ef(p)[:256] for p in lags[t]], axis=1))
    m = np.zeros((512, 128))
    for p in range(2, 257):
        tt, l = where[int(rl[256 + p])]
        assert tt == 2
        m[:, l] += ef(p) * (0.5 if p == 256 else 1.0)
    add("B1", m)
    assert rl[257] == 256
    hf.append(ef(1))
    for tau, lg in _SEL.items():
        parts = [p for p in _PARTS if p[0] == {3: 4, 4: 8}.get(tau)]
        blk = []
        for st, w, p0, p1 in parts:
            nr = 128 // st
            dm = np.zeros((4 * nr, 128))
            for pc in range(p0, p1 + 1, st):
                lag, odd = 256 * (w - 1) + pc, (pc // st) % 2
                assert all(int(rl[lag + d]) == lag for d in range(odd - st // 2, st // 2 + 1 - odd)
                           if p0 < pc + d < p1 and lag + d < L)
                tt, l = where[lag]
                if tt != tau:
                    assert pc == p0
                    continue
                v = ef(pc) * (0.5 if pc in (p0, p1) else 1.0)
                dm[2 * nr * odd:2 * nr * odd + nr, l] += v[0:nr]
                dm[2 * nr * odd + nr:2 * nr * odd + 2 * nr, l] += v[64:64 + nr]
            blk.append(dm)
        sel = np.zeros((16 * ((len(lg) + 1) // 2), 128))
        for j, lag in enumerate(lg):
            assert where[lag][0] == tau
            sel[8 * j:8 * j + 8, where[lag][1]] = 1.0
        add(("D", tau), np.concatenate([sel] + blk, axis=0))
        off["Dn", tau] = rows[-1].shape[0]
    for st in (4, 8):
        ho = 1 + 2 * sum(np.cos(th * d) for d in range(1, st // 2))
        off["T", st] = sum(x.shape[0] for x in hf)
        hf += [ho + 2 * np.cos(th * (st // 2)), ho * (-1.0) ** ((np.arange(256) % 64) // (128 // st)),
               sum(np.sin(th * d) for d in range(1, st // 2 + 1))]
    pos = np.arange(128)
    tc = th[8 * (pos // 16) + pos % 8]
    for c in range(4):
        a = tc[None, :] * (256 + 4 * np.arange(64) + c)[:, None]
        add(("I", c), np.where(pos[None, :] % 16 < 8, np.cos(a), -np.sin(a)) / 256.0)
    fk = _pack_np(np.concatenate(rows, axis=0))
    off["F32"] = fk.shape[0]
    hf = np.repeat(np.concatenate(hf)[:, None], 128, axis=1).astype(np.float32)
    big = np.concatenate([fk, hf.view(np.uint32)], axis=0)
    fu = []
    for par in range(2):
        a = th[:128, None] * (2 * pos + par)[None, :]
        fu.append(_pack_np(np.concatenate([np.cos(a), -np.sin(a)], axis=0)))
    zero = np.zeros((8, 128), np.uint32)
    small = np.concatenate([zero, zero, np.broadcast_to(np.arange(128) < 64, (8, 128)).astype(np.uint32),
                            np.broadcast_to(np.arange(8)[:, None] < 4, (8, 128)).astype(np.uint32)] + fu + [zero], axis=0)
    return off, big, small


class _Packed:
    def __init__(self, ref):
        self.ref = ref

    def __getitem__(self, idx):
        return pltpu.bitcast(self.ref[idx[0].start // 2:idx[0].stop // 2, idx[1]], bf16)

    def __setitem__(self, idx, v):
        self.ref[idx[0].start // 2:idx[0].stop // 2, idx[1]] = pltpu.bitcast(v.astype(bf16), u32)


class _Words:
    def __init__(self, ref):
        self.ref = ref

    def __getitem__(self, idx):
        return pltpu.bitcast(self.ref[2 * idx[0].start:2 * idx[0].stop, idx[1]], u32)

    def __setitem__(self, idx, v):
        self.ref[2 * idx[0].start:2 * idx[0].stop, idx[1]] = pltpu.bitcast(v, bf16)


class _Ctx:
    pass


def _nt(a, b):
    return jax.lax.dot_general(a, b, (((1,), (1,)), ((), ())), preferred_element_type=f32)


def _dot(a, b):
    return jnp.dot(a, b, preferred_element_type=f32)


def _cat(xs, axis):
    return jnp.concatenate(xs, axis=axis)


def _zip2(a, b):
    return pltpu.pack_elementwise([a, b], packed_dtype=bf16)


def _even_odd(w):
    return pltpu.bitcast(w << 16, f32), pltpu.bitcast(w & jnp.uint32(0xFFFF0000), f32)


def _cis(mag, th):
    kf = jnp.floor(th * (2.0 / np.pi) + 0.5)
    k = kf.astype(i32)
    r = ((th - kf * 1.5703125) - kf * 4.837512969970703125e-4) - kf * 7.54978995489188216e-8
    r = jnp.minimum(jnp.maximum(r, -1.0), 1.0)
    r2 = r * r
    s = r + r * (r2 * (-1.6666654611e-1 + r2 * (8.3321608736e-3 + r2 * -1.9515295891e-4)))
    c = 1.0 + r2 * (-0.5 + r2 * (4.166664568298827e-2 + r2 * (-1.388731625493765e-3 + r2 * 2.443315711809948e-5)))
    swap = (k & 1) == 1
    mb = pltpu.bitcast(mag, i32)
    ms = pltpu.bitcast(mb ^ ((k & 2) << 30), f32)
    mc = pltpu.bitcast(mb ^ (((k + 1) & 2) << 30), f32)
    return mc * jnp.where(swap, s, c), ms * jnp.where(swap, c, s)


def _cmul(a, b):
    return a[0] * b[0] - a[1] * b[1], a[0] * b[1] + a[1] * b[0]


def _cmulc(a, b):
    return a[0] * b[0] + a[1] * b[1], a[1] * b[0] - a[0] * b[1]


def _csq(a):
    return a[0] * a[0] - a[1] * a[1], (a[0] + a[0]) * a[1]


def tl(i, n=1):
    return slice(128 * i, 128 * (i + n))


def rs(a, n):
    return slice(a, a + n)


def _kernel(x_hbm, are_h, aim_h, bre_h, bim_h, cre_h, cim_h, ldt_h, dsk_h, wg_h, wu_h, wd_h,
            big_h, sm_h, o_hbm,
            x_v, par_v, ldt_v, dsk_v, wg_v, wu_v, wd_v, big_v, sm_v, coef_s, zw_s, xn_u, xa_u, ha_u,
            wt_u, wdt_u, u_s, xs_u, es_u, kc_s, kw_s, kd_s, y_u, o_s, dum_v, sems):
    off = _consts()[0]
    xn_s, xa_s, ha_s, wt_s, wdt_s, xs_s, es_s, y_s, big_s, sm_s = [
        _Packed(r) for r in (xn_u, xa_u, ha_u, wt_u, wdt_u, xs_u, es_u, y_u, big_v, sm_v)]
    x_u, wg_u, wu_u, wd_u, o_u = [_Words(r) for r in (x_v, wg_v, wu_v, wd_v, o_s)]
    AL = slice(None)
    nsem = [0]

    def grp(pairs):
        nsem[0] += 1
        return [pltpu.make_async_copy(a, b, sems.at[nsem[0] - 1]) for a, b in pairs]

    def cf(r0, n):
        return pltpu.bitcast(big_v[rs(off["F32"] + r0, n), :], f32)

    def mk(paced=True):
        c = _Ctx()
        c.never = (sm_v[0:8, :] != 0) if paced else None
        c.tok = c.xt = None
        c.cnt = 0
        return c

    def tie(c, v, tok):
        if tok is None or c.never is None:
            return v
        if tok.dtype != v.dtype:
            tok = pltpu.bitcast(tok, v.dtype)
        h = jnp.where(c.never, tok, v[:, :128])
        return h if v.shape[1] == 128 else _cat([h, v[:, 128:]], 1)

    def a0(c, ct, nc):
        cs = tl(ct)
        dt = jnp.exp(ldt_v[...].astype(f32).reshape(1, D)[:, cs]).astype(bf16).astype(f32)
        outs = [[], [], [], []]
        k0 = None
        toks = [c.tok] * nc
        for i in range(N // 8):
            ld = lambda q: par_v[q, 8 * i:8 * i + 8, cs].astype(f32)
            tk = toks[i % nc]
            zr, zi = _cis(jnp.exp(dt * ld(0)), tie(c, dt * ld(1), tk))
            cb = _cmul((ld(4), ld(5)), (tie(c, ld(2), tk), tie(c, ld(3), tk)))
            wr, wi = dt * cb[0], dt * cb[1]
            k0 = wr if k0 is None else k0 + wr
            toks[i % nc] = zr
            for o, v in zip(outs, (zr, zi, wr, wi)):
                o.append(v)
        c.tok = toks[-1]
        coef_s[:, cs] = jnp.broadcast_to(
            jnp.sum(k0, axis=0, keepdims=True) + dsk_v[...].astype(f32).reshape(1, D)[:, cs], (8, 128))
        hi = [outs[0][16:] * 2, outs[1][16:] * 2, [-v for v in outs[3][16:]] + outs[2][16:], outs[2][16:] + outs[3][16:]]
        for q in range(4):
            for h, v in enumerate((_cat(outs[q][:16], 0).T, _cat(hi[q], 0).T)):
                zw_s[q, cs, tl(h)] = v
                c.xt = v[120:128] if c.xt is None else c.xt + v[120:128]

    def ln(c, t, toks):
        for i in range(8):
            eo = ([], [])
            for g in range(2):
                wr = rs(128 * t + 16 * i + 8 * g, 8)
                for hh, xx in enumerate(_even_odd(x_u[wr, AL])):
                    ci = (4 * i + 2 * g + hh) % len(toks)
                    xx = tie(c, xx, toks[ci])
                    mu = jnp.sum(xx, axis=1, keepdims=True) * (1.0 / D)
                    var = jnp.maximum(jnp.sum(xx * xx, axis=1, keepdims=True) * (1.0 / D) - mu * mu, 0.0)
                    if c.never is not None:
                        xx = pltpu.unpack_elementwise(x_u[wr, AL], index=hh, packed_dtype=bf16, unpacked_dtype=f32)
                    xn = (xx - mu) * jax.lax.rsqrt(var + 1e-5)
                    toks[ci] = xn[:, :128]
                    eo[hh].append(xn)
            top, bot = _cat(eo[0], 0), _cat(eo[1], 0)
            xn_s[rs(RB * t + 16 * i, 16), AL] = top
            xn_s[rs(RB * t + 128 + 16 * i, 16), AL] = bot
            a11, a12, a21, a22 = top[:, 0:256], top[:, 256:512], bot[:, 0:256], bot[:, 256:512]
            for q, v in enumerate((a11 + a22, a21 + a22, a11 + a12, a21 - a11, a12 - a22)):
                xa_s[rs(128 * t + 16 * i, 16), tl(2 * q, 2)] = v

    def bcomb(c, src, dst, kw, n1, dcol, srow):
        for i in range(kw // 8):
            ws = [tie(c, src[rs(srow(h, i), 8), tl(n)], c.tok) for h in range(2) for n in (n1, n1 + 1)]
            q = [_even_odd(w) for w in ws]
            res = []
            for p in range(2):
                b11, b12, b21, b22 = (v[p] for v in q)
                res.append((b11 + b22, b12 - b22, b21 - b11, b11 + b12, b21 + b22))
            pks = [_zip2(res[0][j], res[1][j]) for j in range(5)] + [ws[0], ws[3]]
            for j, pk in enumerate(pks):
                dst[rs(j * kw + 8 * i, 8), tl(dcol)] = pk
            c.tok = res[0][1] + (res[0][0] + pltpu.bitcast(pks[4], f32))

    def wcomb(c, ck):
        for m, src in enumerate((wg_u, wu_u)):
            bcomb(c, src, wt_u, 128, 2 * ck, 2 * ck + m, lambda h, i: 128 * h + 8 * i)
            for i in range(8):
                ws = [tie(c, src[rs(256 + 8 * i, 8), tl(n)], c.tok) for n in (2 * ck, 2 * ck + 1)]
                q = [_even_odd(w) for w in ws]
                c.tok = q[0][0] + q[1][0]
                for j, w in enumerate((_zip2(c.tok, q[0][1] + q[1][1]), ws[0], ws[1])):
                    wt_u[rs(896 + 64 * j + 8 * i, 8), tl(2 * ck + m)] = w

    def wdcomb(c, pr):
        srow = lambda h, i: 128 * (i // 8) + 64 * h + 8 * (i % 8)
        bcomb(c, wd_u, wdt_u, 384, 2 * pr, pr, srow)
        for i in range(48):
            w = tie(c, wd_u[rs(srow(pr, i), 8), tl(4)], c.tok)
            wdt_u[rs(7 * 384 + 8 * i, 8), tl(pr)] = w
            c.tok = pltpu.bitcast(w, f32) + 1.0

    def xe(c, o):
        lo64, slo = sm_v[16:24, :] != 0, sm_v[24:32, :] != 0
        rolled = {}

        def roll4(v):
            if id(v) not in rolled:
                rolled[id(v)] = (v, pltpu.roll(v, 4, 0))
            return rolled[id(v)][1]

        def mix(a, b, g):
            return tuple(jnp.where(slo, u, roll4(v)) if g == 0 else jnp.where(slo, roll4(u), v) for u, v in zip(a, b))

        def tiec(v, tok):
            return tuple(tie(c, u, tok) for u in v)

        l01 = jnp.where(lo64, 1.0, 0.0).astype(f32)
        prep = []
        tok = c.tok
        for h in range(2):
            z = tiec((zw_s[0, rs(8 * o, 8), tl(h)], zw_s[1, rs(8 * o, 8), tl(h)]), tok)
            w = (zw_s[2, rs(8 * o, 8), tl(h)], zw_s[3, rs(8 * o, 8), tl(h)])
            pw = {1: z}
            e = 1
            while e < 512:
                pw[2 * e] = _csq(pw[e])
                e *= 2
                if e == 2:
                    wz = _cmul(w, z)
                if e == 8:
                    wz5 = _cmul(wz, pw[4])
            p772 = _cmul(_cmul(pw[256], pw[4]), pw[512])
            er, ei = pw[128]
            if h == 0:
                one, eb = (jnp.ones((8, 128), f32), jnp.zeros((8, 128), f32)), (er, -ei)
            else:
                one, eb = (1.0 - l01, l01), (jnp.where(lo64, ei, er), jnp.where(lo64, er, -ei))
            prep.append((z, wz, wz5, pw[256], p772, pw[8], one, eb))
            if c.xps:
                tok = p772[0]
        tok = p772[0]
        for g in range(2):
            def put(ref, n, lst, h):
                i = len(lst) - 2
                if i % 2 == 0:
                    b0 = (2 * (o % XR) + g) * 8 * n + 8 * i
                    for q, cb in ([(0, 0), (1, 1)] if h == 0 else [(1, 2)]):
                        ref[rs(b0, 16), tl(cb)] = _cat([lst[i][q], lst[i + 1][q]], 0)

            def xseg(h, tok):
                z, wz, wz5, p256, p772 = prep[h][:5]
                xs = [tiec(mix(wz, wz5, g), tok)]
                a1 = mix(z, z, g)
                a256 = am = None
                for src in (0, 1, 2, 1, 3, 5, 6, 7, 8):
                    if len(xs) == 3:
                        a256 = mix(p256, p256, g)
                    if len(xs) == 6:
                        am = mix(p772, p256, g)
                    xs.append(_cmul(xs[src], a1 if len(xs) < 4 else (am if len(xs) == 8 else a256)))
                    put(xs_s, 10, xs, h)
                return xs[-1][1]

            def eseg(hs, tok):
                es, a8 = {}, {}
                for h in hs:
                    p8, one, eb = prep[h][5:]
                    a8[h] = mix(p8, p8, g)
                    es[h] = [tiec(tuple(jnp.where(slo, u, roll4(v) if g == 0 else v) for u, v in zip(one, eb)), tok)]
                if 1 in hs:
                    ra, rb = a8[1][0] + a8[1][0], a8[1][0] * a8[1][0] + a8[1][1] * a8[1][1]
                for v in range(15):
                    for h in hs:
                        if h == 0 or v == 0:
                            es[h].append(_cmulc(es[h][-1], a8[h]))
                        else:
                            es[h].append((None, ra * es[h][-1][1] - rb * es[h][-2][1]))
                        put(es_s, 16, es[h], h)
                return es[hs[0]][-1][1]

            tok = xseg(0, tok)
            tok = eseg([1], eseg([0], tok)) if (c.xs2 and (2 * o + g) % c.xs2 == 0) else eseg([0, 1], tok)
            tok = xseg(1, tok)
        c.tok = tok

    def c2(c, unit):
        ct, p = divmod(unit, 8)
        ys, gs = {}, {}
        for cl in (0, 2, 1, 3):
            rws = rs(64 * cl + 8 * p, 8)
            pos = cl in (0, 3)

            def kpart(pt, s):
                ht = lambda q: cf(off["T", pt[0]] + 256 * q + 64 * cl + 8 * p, 8)
                kd = lambda q: kd_s[ct, _KD[pt, q] + (p % (16 // pt[0]) if q in range(6) else 0)]
                half = pt[3] - pt[2] == 256
                if s == 0:
                    kv = ht(0) * kd(4) + ht(1) * kd(5)
                    return kv if not half else (kv + ht(2) * kd("b") if pos else kv - ht(2) * kd("b"))
                q = (s - 1) ^ (not pos)
                kv, tv = ht(0) * kd(q) + ht(1) * kd(2 + q), ht(2) * kd("a-b" if half and q else "a+b")
                return kv - tv if s == 1 else kv + tv

            k1, ri = None, {}
            for s in range(3):
                U, K, out = [], [], []
                for i in range(NS):
                    U.append(u_s[ct, 0, i, rws, :] + u_s[ct, 1, i, rws, :] if s == 0 else u_s[ct, s - 1, i, rws, :])
                    ks = [kpart(pt, s) for pt in _PARTS if pt[1] == i]
                    if i < 3:
                        ks.append((kw_s[ct, 0, i, rws, :] + kw_s[ct, 1, i, rws, :]) * (-0.5) if s == 0
                                  else kw_s[ct, s - 1, i, rws, :])
                    K.append(ks[0] if len(ks) == 1 else ks[0] + ks[1])
                    ms = list(range(1, i)) + ([0, i] if i else [0])
                    a = tie(c, k1[i] if s else K[ms[0]] * U[i - ms[0]], c.tok)
                    ms = ms if s else ms[1:]
                    while ms:
                        c.cnt += 1
                        pr = K[ms[0]] * U[i - ms[0]]
                        if c.cnt % c.ps[1] < c.ps[0] and len(ms) > 1 and (c.jit or not (s == 2 and cl == 3)):
                            pr = pr + K[ms[1]] * U[i - ms[1]]
                            ms = ms[1:]
                        ms = ms[1:]
                        a = a + pr
                    c.tok = a
                    out.append(a)
                    if s == 2 and cl >= 2:
                        yr, yi, zr, zi = ys[cl - 2][2][i], ys[cl - 2][1][i], a, ri[1][i]
                        g = (yr + zr, yi - zi, yr - zr, yi + zi)
                        if cl == 2:
                            gs[i] = g
                            c.tok = a if c.jit else g[2]
                        else:
                            e = gs[i]
                            hs = ((e[0] + g[0], e[1] - g[1]), (e[2] - g[3], e[3] - g[2]),
                                  (e[0] - g[0], e[1] + g[1]), (e[2] + g[3], e[3] + g[2]))
                            for q, h in enumerate(hs):
                                y_s[rs(512 * ct + 128 * q + 16 * p, 16), tl(i)] = _cat(h, 0)
                            c.tok = a if c.jit else hs[3][1] + hs[0][0]
                if s == 0:
                    k1 = out
                else:
                    ri[s] = out
            ys[cl] = ri

    queue = []

    def hook():
        if queue:
            queue.pop(0)()

    def ffn1(t, ck, strassen=True):
        top, bot = rs(RB * t, 128), rs(RB * t + 128, 128)
        if strassen:
            cw = tl(2 * ck, 2)
            sa = lambda q: xa_s[rs(128 * t, 128), tl(2 * q, 2)]
            tb = lambda q: wt_s[rs(256 * q, 256), cw]
            tk, k3a, k3b = (wt_s[rs(1792 + 128 * j, 128), cw] for j in range(3))
            m4 = _dot(xn_s[bot, tl(2, 2)], tb(2))
            hook()
            m2 = _dot(_cat([sa(1), xn_s[bot, tl(4)]], 1), _cat([tb(5), k3a], 0))
            c21 = m2 + m4
            hook()
            m5 = _dot(_cat([sa(2), xn_s[top, tl(4)]], 1), _cat([tb(6), k3b], 0))
            hook()
            m3 = _dot(xn_s[top, tl(0, 2)], tb(1))
            c12 = m3 + m5
            hook()
            m1 = _dot(sa(0), tb(0))
            hook()
            m7 = _dot(_cat([sa(4), xn_s[top, tl(4)]], 1), _cat([tb(4), tk], 0))
            hook()
            m6 = _dot(_cat([sa(3), xn_s[bot, tl(4)]], 1), _cat([tb(3), tk], 0))
            c11, c22 = m7 + (m1 + (m4 - m5)), m6 + (m1 + (m3 - m2))
        else:
            xn = xn_s[rs(RB * t, RB), AL]
            r1 = _dot(xn, _cat([wg_v[:, tl(2 * ck)], wu_v[:, tl(2 * ck)]], 1))
            r2 = _dot(xn, _cat([wg_v[:, tl(2 * ck + 1)], wu_v[:, tl(2 * ck + 1)]], 1))
            c11, c21, c12, c22 = r1[:128], r1[128:], r2[:128], r2[128:]
        h11, h12, h21, h22 = (v[:, :128] * v[:, 128:] for v in (c11, c12, c21, c22))
        for q, v in enumerate((h11, h12, h21, h22, h11 + h22, h21 + h22, h11 + h12, h21 - h11, h12 - h22)):
            ha_s[rs(128 * t, 128), tl(6 * q + ck)] = v
        return c21[0:8, 0:128]

    def ufwd(t):
        for c0, n in ((0, 2), (2, 2), (4, 1)):
            e = _dot(sm_s[64:320, AL], xn_s[rs(RB * t, 128), tl(c0, n)])
            o = _dot(sm_s[320:576, AL], xn_s[rs(RB * t + 128, 128), tl(c0, n)])
            for j in range(n):
                er, ei, or_, oi = e[:128, tl(j)], e[128:, tl(j)], o[:128, tl(j)], o[128:, tl(j)]
                u_s[c0 + j, 0, t, 0:128], u_s[c0 + j, 0, t, 128:256] = er + or_, er - or_
                u_s[c0 + j, 1, t, 0:128], u_s[c0 + j, 1, t, 128:256] = ei + oi, oi - ei
            if c0 == 0:
                yield

    def kmm(o):
        lane = jax.lax.broadcasted_iota(i32, (8, 128), 1)
        sub = jax.lax.broadcasted_iota(i32, (8, 128), 0)
        slo = sub < 4
        res = [_nt(xs_s[rs(80 * q, 80), AL], es_s[rs(128 * q, 128), AL]) for q in (2 * (o % XR), 2 * (o % XR) + 1)]
        dk = (lane - sub) & 3

        def merge(r, vs):
            out = None
            for k in reversed(range(len(vs))):
                src = r[8 * vs[k]:8 * vs[k] + 8, :]
                if k:
                    src = pltpu.roll(src, k, 1)
                out = src if out is None else jnp.where(dk == k, src, out)
            return out

        def derot(x):
            x = jnp.where((sub & 1) == 1, pltpu.roll(x, 127, 1), x)
            return jnp.where((sub & 2) == 2, pltpu.roll(x, 126, 1), x)

        ts = []
        for vs, sh in (([0, 1, 2, 3], 1), ([4, 5, 6, 7], 2), ([8, 9], 2)):
            a, b = merge(res[0], vs), merge(res[1], vs)
            a, b = jnp.where(slo, a, pltpu.roll(b, 4, 0)), pltpu.roll(jnp.where(slo, pltpu.roll(a, 4, 0), b), sh, 1)
            m = (dk & sh) == 0
            ts += [jnp.where(m, a, b), jnp.where(m, b, a)]
        for i in range(5):
            kc_s[i, rs(8 * o, 8), :] = derot(ts[i])

    def kfwd(ct):
        kt = lambda tau: kc_s[tau, tl(ct), :].astype(bf16)
        kv = {}
        for tau, lg in _SEL.items():
            v = _nt(big_s[rs(off["D", tau], off["Dn", tau]), AL], kt(tau))
            kv.update({lag: v[rs(8 * j, 8)] for j, lag in enumerate(lg)})
            r0 = 16 * ((len(lg) + 1) // 2)
            for pt in [p for p in _PARTS if p[0] == {3: 4, 4: 8}.get(tau)]:
                st, w, p0, p1 = pt
                n = 16 // st
                d = [[v[rs(r0 + 8 * (n * q + j), 8)] for j in range(n)] for q in range(4)]
                r0 += 32 * n
                vl, vr = kv[256 * (w - 1) + p0], kv[256 * (w - 1) + p1]
                if 256 * (w - 1) + p0 not in lg:
                    hv = vl * 0.5
                    d[0], d[1] = [x - hv for x in d[0]], [x + hv if p0 else x - hv for x in d[1]]
                d += [[(x + y) * (-0.5) for x, y in zip(d[q], d[q + 1])] for q in (0, 2)]
                for q in range(6):
                    for j in range(n):
                        kd_s[ct, _KD[pt, q] + j] = d[q][j]
                if p1 - p0 == 512:
                    kd_s[ct, _KD[pt, "a+b"]] = vl + vr
                else:
                    a, b = (vr, -vl) if p0 else (vl, vr)
                    kd_s[ct, _KD[pt, "a+b"]], kd_s[ct, _KD[pt, "a-b"]], kd_s[ct, _KD[pt, "b"]] = a + b, a - b, b
        yield
        for cb in range(2):
            od, ev = (_nt(big_s[rs(off["B0", t] + 128 * cb, 128), AL], kt(t)) for t in (0, 1))
            sm, df = ev + od, ev - od
            for cl, (e0, f0) in ((cb, (sm[:64], sm[64:])), (cb + 2, (df[64:], df[:64]))):
                pos, rw = cl in (0, 3), rs(64 * cl, 64)
                v = _nt(big_s[rs(off["B1"] + 128 * cl, 128), AL], kt(2)) + cf(128 * cl, 128) * _cat([kv[256]] * 16, 0)
                e1, f1 = v[:64], v[64:]
                kw_s[ct, 0, 0, rw], kw_s[ct, 1, 0, rw] = (f0, -e0) if pos else (-f0, e0)
                kw_s[ct, 0, 1, rw], kw_s[ct, 1, 1, rw] = (e0 + f1, f0 - e1) if pos else (e0 - f1, f0 + e1)
                kw_s[ct, 0, 2, rw], kw_s[ct, 1, 2, rw] = e1, f1
            yield

    def inv(ct, t):
        y = [_dot(big_s[rs(off["I", q], 64), AL], y_s[rs(512 * ct + 128 * q, 128), tl(t)]) for q in range(4)]
        return _zip2(y[0], y[2]), _zip2(y[1], y[3])

    def finish(ct, t, dt_, db_):
        y = inv(ct, t)
        xs = _even_odd(x_u[rs(128 * t, 128), tl(ct)])
        res = []
        for h, dn in enumerate((dt_, db_)):
            yy = pltpu.bitcast(y[h], bf16).astype(f32)
            xn = xn_s[rs(RB * t + 128 * h, 128), tl(ct)].astype(f32)
            res.append(xs[h] + (xn * coef_s[0:1, tl(ct)] + dn) + yy)
        o_u[rs((ct * L + RB * t) // 2, 128), AL] = _zip2(*res)
        c_out[ct * NS + t].start()

    pend = {}

    def flush(ct, t):
        finish(ct, t, *pend.pop((ct, t)))

    def down4(t):
        dn = _dot(_cat([ha_s[rs(128 * t, 128), 0:1536], ha_s[rs(128 * t, 128), 1536:3072]], 0),
                  _cat([wdt_s[5376:6144, tl(0)], wdt_s[5376:6144, tl(1)]], 0))
        pend[4, t] = (dn[:128], dn[128:])

    def down_pair(pr, t):
        m = {}
        for k, (a, b) in ((1, (4, 0)), (4, (3, 2)), (5, (6, 6)), (7, (8, 4)), (2, (5, 5)), (3, (0, 1)), (6, (7, 3))):
            m[k] = _dot(ha_s[rs(128 * t, 128), tl(6 * a, 6)], wdt_s[rs(768 * b, 768), tl(pr)])
            if k == 2:
                pend[2 * pr, t] = (m[7] + m[1] + m[4] - m[5], m[2] + m[4])
            if k == 6:
                pend[2 * pr + 1, t] = (m[3] + m[5], m[6] + m[1] - m[2] + m[3])
            yield

    pars = (are_h, aim_h, bre_h, bim_h, cre_h, cim_h)
    par = lambda a, n: [(p.at[:, tl(a, n)], par_v.at[i, :, tl(a, n)]) for i, p in enumerate(pars)]
    xr = lambda a, b: [(x_hbm.at[a * RB:b * RB], x_v.at[a * RB:b * RB])]
    wch = lambda a, n: [(h.at[:, tl(2 * a, 2 * n)], v.at[:, tl(2 * a, 2 * n)]) for h, v in ((wg_h, wg_v), (wu_h, wu_v))]
    dum = lambda i: [(sm_h.at[0:8], dum_v.at[8 * i:8 * i + 8])]
    G = [grp(p) for p in (
        xr(0, 1), [(sm_h, sm_v)] + xr(1, 2), wch(0, 1), wch(1, 1) + xr(2, 3),
        wch(2, 1) + xr(3, 4) + par(0, 1) + [(ldt_h, ldt_v), (dsk_h, dsk_v)], par(1, 1) + wch(3, 3),
        par(2, 3) + xr(4, 8), [(big_h, big_v), (wd_h, wd_v)], dum(0), dum(1), dum(2))]
    c_out = grp([(o_s.at[rs(ct * L + RB * t, RB)], o_hbm.at[rs(RB * t, RB), tl(ct)])
                 for ct in range(NCT) for t in range(NS)])

    def wait(cs):
        for cc in cs:
            cc.wait()

    def run_all(gen):
        for _ in gen:
            pass

    def part(c, main=(), km=(), uf=(), kf=(), wc=(), wdc=(), lns=(), a0s=(), xes=(), c2s=(),
             late=None, nw=4, nk=None, xps=1, ps=(1, 1), xs2=0, nc=2, jit=0, wcj=(), fine=1):
        c.xps, c.ps, c.xs2, c.jit = xps, ps, xs2, jit
        if wcj:
            keep = c.tok, c.never
            c.tok, c.never = None, sm_v[288:296, :] != 0
            for ck in wcj:
                wcomb(c, ck)
            c.tok, c.never = keep
        for ck in wc:
            wcomb(c, ck)
        for pr in wdc:
            wdcomb(c, pr)
        for o in xes:
            xe(c, o)
        for un in c2s:
            c2(c, un)
        extra = []
        for gen, n in [(ufwd(t), 2) for t in uf] + [(kfwd(ct), 3) for ct in kf]:
            extra += [functools.partial(next, gen, None)] * n
        nm, kms, mt = len(main), list(km), []
        nkk = nk if nk is not None else nm - 1
        for i, fn in enumerate(main):
            if i < nkk:
                queue.extend(functools.partial(kmm, o) for o in kms[i * len(kms) // nkk:(i + 1) * len(kms) // nkk])
            queue.extend(extra[i * len(extra) // nm:(i + 1) * len(extra) // nm])
            while len(queue) > (6 if fine else 0):
                hook()
            mt.append(fn())
            while queue:
                hook()
        if a0s or lns:
            keep = c.tok, c.never
            c.tok, c.never = (None if late is None else mt[late]), sm_v[8:16, :] != 0
            for ct in a0s:
                a0(c, ct, nc)
            toks = [c.xt if a0s else c.tok] * nw
            for q in range(1, nw if toks[0] is not None else 0):
                toks[q] = functools.reduce(lambda a, _: a + 1.0, range(20), toks[q - 1])
            for t in lns:
                ln(c, t, toks)
            c.tok, c.never = keep

    def block(waits, *parts, end=()):
        def run():
            wait(waits)
            c = mk()
            for p in (parts[0]() if callable(parts[0]) else parts):
                part(c, **p)
            wait(end)
        return run

    for g in G:
        for cc in g:
            cc.start()
    flag = jax.lax.fori_loop(0, 3, lambda i, a: a + i, 0)
    wait(G[0])
    ln(mk(False), 0, [None])

    def p1():
        wait(G[1])
        run_all(ufwd(0))
        ln(mk(False), 1, [None])
        run_all(ufwd(1))

    R, P = range, functools.partial
    it = [P(ffn1, t, ck) for t, ck in ([(t, ck) for t in (2, 3) for ck in R(3)] + [(t, ck) for t in R(4) for ck in R(3, 6)]
                                       + [(t, ck) for t in R(4, 8) for ck in R(6)])]

    def pairs(pr, inline):
        out = []
        fl = lambda ct, t: [P(flush, ct, t)] if inline and t >= 0 else []
        for t in R(NS):
            d = [P(next, down_pair(pr, t), None)] * 7
            out += d[:1] + fl(2 * pr, t - 1) + d[1:3] + fl(2 * pr + 1, t - 1) + d[3:]
        return out[:-2] + fl(2 * pr, NS - 1) + out[-2:] + fl(2 * pr + 1, NS - 1)

    def yparts():
        m = pairs(0, True)
        return [dict(main=m[:56], km=R(64, 80), nk=40, c2s=R(16, 27), ps=(0, 1), fine=0),
                dict(main=m[56:], kf=[4], fine=0)]

    def zparts():
        m = pairs(1, False)
        for t in R(NS):
            m += [P(down4, t)] + [P(flush, ct, t) for ct in (2, 3) if t < 6] + [P(flush, 4, t)]
            if 3 <= t <= 6:
                m += [P(flush, 2 + (t + 1) % 2, 6 + (t - 3) // 2)]
        return [dict(main=m, c2s=R(27, 40), ps=(2, 3), jit=1)]

    blocks = [
        p1,
        block(G[2], dict(main=[P(ffn1, 0, 0, False), P(ffn1, 1, 0)], wcj=[0])),
        block(G[3], dict(main=[P(ffn1, 0, 1, False), P(ffn1, 1, 1)], wcj=[1], lns=[2], nw=6)),
        block(G[4], dict(main=it[0:1] + [P(ffn1, 0, 2), P(ffn1, 1, 2)] + it[1:2], uf=[2], wcj=[2], a0s=[0], lns=[3], nc=1, nw=3)),
        block(G[5], dict(main=it[2:6], uf=[3], wc=[3, 4, 5], xes=R(0, 10), a0s=[1], xps=0, nc=2)),
        block(G[6], dict(main=it[6:18], km=R(0, 10), xes=R(10, 32), lns=R(4, 8), a0s=[2, 3], late=5, nk=2,
                         nw=5, xps=0, nc=2)),
        block(G[7], dict(main=it[18:24], km=R(10, 32), nk=5, uf=R(4, 8), wdc=[0, 1], xes=R(32, 64),
                         xs2=2),
              dict(main=it[24:28], kf=[0, 1], a0s=[4], late=2, nc=1)),
        block(G[8], dict(main=it[28:40], km=R(32, 64), nk=6, xes=R(64, 80), xs2=2, c2s=R(0, 16), ps=(1, 3)),
              dict(main=it[40:42], kf=[2, 3])),
        block(G[9], yparts),
        block(G[10], zparts, end=c_out),
    ]
    for i, fn in enumerate(blocks):
        pl.when(flag > -i)(fn)


@jax.jit
def pallas_parallel_sum__ssm_conv_s4__glu_gated_bilinear__prompt_kernel(A_u, A_A_re, A_A_im, A_B_re, A_B_im, A_C_re, A_C_im, A_log_dt, A_Dskip, B_x, B_w_gate, B_w_up, B_w_down):
    _, big, small = _consts()
    hbm = pl.BlockSpec(memory_space=pltpu.HBM)
    out = pl.pallas_call(
        _kernel,
        in_specs=[hbm] * 14,
        out_specs=hbm,
        out_shape=jax.ShapeDtypeStruct((L, D), bf16),
        scratch_shapes=[
            pltpu.VMEM((L, D), bf16),
            pltpu.VMEM((6, N, D), bf16),
            pltpu.VMEM((D,), bf16), pltpu.VMEM((D,), bf16),
            pltpu.VMEM((D, F), bf16), pltpu.VMEM((D, F), bf16), pltpu.VMEM((F, D), bf16),
            pltpu.VMEM(big.shape, u32), pltpu.VMEM(small.shape, u32),
            pltpu.VMEM((8, D), f32),
            pltpu.VMEM((4, D, 256), f32),
            pltpu.VMEM((L // 2, D), u32),
            pltpu.VMEM((L // 4, 1280), u32),
            pltpu.VMEM((L // 4, 9 * 768), u32),
            pltpu.VMEM((1088, F), u32),
            pltpu.VMEM((8 * 384, 256), u32),
            pltpu.VMEM((NCT, 2, NS, 256, 128), f32),
            pltpu.VMEM((2 * XR * 40, 384), u32),
            pltpu.VMEM((2 * XR * 64, 384), u32),
            pltpu.VMEM((5, D, 128), f32),
            pltpu.VMEM((NCT, 2, 3, 256, 128), f32),
            pltpu.VMEM((NCT, _KD["n"], 8, 128), f32),
            pltpu.VMEM((NCT * 256, NS * 128), u32),
            pltpu.VMEM((NCT * L, 128), bf16),
            pltpu.VMEM((24, 128), u32),
            pltpu.SemaphoreType.DMA((12,)),
        ],
        compiler_params=pltpu.CompilerParams(vmem_limit_bytes=110 * 1024 * 1024),
    )(A_u.reshape(L, D), A_A_re.T, A_A_im.T, A_B_re.T, A_B_im.T, A_C_re.T, A_C_im.T, A_log_dt, A_Dskip,
      B_w_gate, B_w_up, B_w_down, jnp.asarray(big), jnp.asarray(small))
    return out.reshape(1, L, D)
```

```python
import functools
import numpy as np
import jax
import jax.numpy as jnp
import jax.experimental.pallas as pl
import jax.experimental.pallas.tpu as pltpu

L, D, N, F = 2048, 640, 192, 1536
RB = 256
NS = L // RB
NCT = D // 128
NCK = 6
XR = 56
f32, bf16, u32, i32 = jnp.float32, jnp.bfloat16, jnp.uint32, jnp.int32

_PARTS = [(4, 2, 256, 512), (4, 3, 0, 512), (4, 4, 0, 256), (8, 4, 256, 512), (8, 5, 0, 512), (8, 6, 0, 512), (8, 7, 0, 512)]
_SEL = {1: [256], 2: [512], 3: [768, 1024], 4: [1280, 1536, 1792, 2048]}
_KD = {}
for _p in _PARTS:
    for _n, _w in [(q, 16 // _p[0]) for q in range(6)] + [("a+b", 1), ("a-b", 1), ("b", 1)]:
        _KD[_p, _n] = _KD.get("n", 0)
        _KD["n"] = _KD.get("n", 0) + _w


def _tile_lags():
    lane = np.arange(128)
    q, k = lane // 4, lane % 4
    j8 = 8 * (q // 2 + 16 * (q % 2))
    t = []
    for a0, a1, sh in (([1, 2, 3, 4], [5, 6, 7, 8], 1), ([258, 260, 516, 772], [262, 264, 520, 776], 2),
                       ([1544, 1800, 0, 0], [1032, 1288, 0, 0], 2)):
        a, b = np.asarray(a0)[k] + j8, np.roll(np.asarray(a1)[k] + j8, sh)
        m = lane % (2 * sh) < sh
        t += [np.where(m, a, b), np.where(m, b, a)]
    return np.stack(t[:5])


def _pack_np(a):
    b = np.asarray(a, np.float32).astype(jnp.bfloat16).view(np.uint16).astype(np.uint32)
    return b[0::2] | (b[1::2] << 16)


@functools.lru_cache(maxsize=None)
def _consts():
    rl = np.arange(L).astype(np.float32).astype(jnp.bfloat16).astype(np.int64)
    lags = _tile_lags()
    where = {int(v): (t, l) for t in range(5) for l, v in enumerate(lags[t])}
    r2 = 2 * np.arange(64)
    th = 2 * np.pi * (np.concatenate([r2, 127 - r2, 255 - r2, 128 + r2]) + 0.5) / 512

    def ef(p):
        re, im = np.cos(th * p).reshape(4, 64), -np.sin(th * p).reshape(4, 64)
        return np.stack([im - re, -(re + im)], axis=1).reshape(512)

    rows, off, hf = [], {}, []

    def add(key, m):
        off[key] = sum(x.shape[0] for x in rows)
        rows.append(m)

    for t in (0, 1):
        add(("B0", t), np.stack([ef(p)[:256] for p in lags[t]], axis=1))
    m = np.zeros((512, 128))
    for p in range(2, 257):
        tt, l = where[int(rl[256 + p])]
        assert tt == 2
        m[:, l] += ef(p) * (0.5 if p == 256 else 1.0)
    add("B1", m)
    assert rl[257] == 256
    hf.append(ef(1))
    for tau, lg in _SEL.items():
        parts = [p for p in _PARTS if p[0] == {3: 4, 4: 8}.get(tau)]
        blk = []
        for st, w, p0, p1 in parts:
            nr = 128 // st
            dm = np.zeros((4 * nr, 128))
            for pc in range(p0, p1 + 1, st):
                lag, odd = 256 * (w - 1) + pc, (pc // st) % 2
                assert all(int(rl[lag + d]) == lag for d in range(odd - st // 2, st // 2 + 1 - odd)
                           if p0 < pc + d < p1 and lag + d < L)
                tt, l = where[lag]
                if tt != tau:
                    assert pc == p0
                    continue
                v = ef(pc) * (0.5 if pc in (p0, p1) else 1.0)
                dm[2 * nr * odd:2 * nr * odd + nr, l] += v[0:nr]
                dm[2 * nr * odd + nr:2 * nr * odd + 2 * nr, l] += v[64:64 + nr]
            blk.append(dm)
        sel = np.zeros((16 * ((len(lg) + 1) // 2), 128))
        for j, lag in enumerate(lg):
            assert where[lag][0] == tau
            sel[8 * j:8 * j + 8, where[lag][1]] = 1.0
        add(("D", tau), np.concatenate([sel] + blk, axis=0))
        off["Dn", tau] = rows[-1].shape[0]
    for st in (4, 8):
        ho = 1 + 2 * sum(np.cos(th * d) for d in range(1, st // 2))
        off["T", st] = sum(x.shape[0] for x in hf)
        hf += [ho + 2 * np.cos(th * (st // 2)), ho * (-1.0) ** ((np.arange(256) % 64) // (128 // st)),
               sum(np.sin(th * d) for d in range(1, st // 2 + 1))]
    pos = np.arange(128)
    tc = th[8 * (pos // 16) + pos % 8]
    for c in range(4):
        a = tc[None, :] * (256 + 4 * np.arange(64) + c)[:, None]
        add(("I", c), np.where(pos[None, :] % 16 < 8, np.cos(a), -np.sin(a)) / 256.0)
    fk = _pack_np(np.concatenate(rows, axis=0))
    off["F32"] = fk.shape[0]
    hf = np.repeat(np.concatenate(hf)[:, None], 128, axis=1).astype(np.float32)
    big = np.concatenate([fk, hf.view(np.uint32)], axis=0)
    fu = []
    for par in range(2):
        a = th[:128, None] * (2 * pos + par)[None, :]
        fu.append(_pack_np(np.concatenate([np.cos(a), -np.sin(a)], axis=0)))
    zero = np.zeros((8, 128), np.uint32)
    small = np.concatenate([zero, zero, np.broadcast_to(np.arange(128) < 64, (8, 128)).astype(np.uint32),
                            np.broadcast_to(np.arange(8)[:, None] < 4, (8, 128)).astype(np.uint32)] + fu + [zero], axis=0)
    return off, big, small


class _Packed:
    def __init__(self, ref):
        self.ref = ref

    def __getitem__(self, idx):
        return pltpu.bitcast(self.ref[idx[0].start // 2:idx[0].stop // 2, idx[1]], bf16)

    def __setitem__(self, idx, v):
        self.ref[idx[0].start // 2:idx[0].stop // 2, idx[1]] = pltpu.bitcast(v.astype(bf16), u32)


class _Words:
    def __init__(self, ref):
        self.ref = ref

    def __getitem__(self, idx):
        return pltpu.bitcast(self.ref[2 * idx[0].start:2 * idx[0].stop, idx[1]], u32)

    def __setitem__(self, idx, v):
        self.ref[2 * idx[0].start:2 * idx[0].stop, idx[1]] = pltpu.bitcast(v, bf16)


class _Ctx:
    pass


def _nt(a, b):
    return jax.lax.dot_general(a, b, (((1,), (1,)), ((), ())), preferred_element_type=f32)


def _dot(a, b):
    return jnp.dot(a, b, preferred_element_type=f32)


def _cat(xs, axis):
    return jnp.concatenate(xs, axis=axis)


def _zip2(a, b):
    return pltpu.pack_elementwise([a, b], packed_dtype=bf16)


def _even_odd(w):
    return pltpu.bitcast(w << 16, f32), pltpu.bitcast(w & jnp.uint32(0xFFFF0000), f32)


def _cis(mag, th):
    kf = jnp.floor(th * (2.0 / np.pi) + 0.5)
    k = kf.astype(i32)
    r = ((th - kf * 1.5703125) - kf * 4.837512969970703125e-4) - kf * 7.54978995489188216e-8
    r = jnp.minimum(jnp.maximum(r, -1.0), 1.0)
    r2 = r * r
    s = r + r * (r2 * (-1.6666654611e-1 + r2 * (8.3321608736e-3 + r2 * -1.9515295891e-4)))
    c = 1.0 + r2 * (-0.5 + r2 * (4.166664568298827e-2 + r2 * (-1.388731625493765e-3 + r2 * 2.443315711809948e-5)))
    swap = (k & 1) == 1
    mb = pltpu.bitcast(mag, i32)
    ms = pltpu.bitcast(mb ^ ((k & 2) << 30), f32)
    mc = pltpu.bitcast(mb ^ (((k + 1) & 2) << 30), f32)
    return mc * jnp.where(swap, s, c), ms * jnp.where(swap, c, s)


def _cmul(a, b):
    return a[0] * b[0] - a[1] * b[1], a[0] * b[1] + a[1] * b[0]


def _cmulc(a, b):
    return a[0] * b[0] + a[1] * b[1], a[1] * b[0] - a[0] * b[1]


def _csq(a):
    return a[0] * a[0] - a[1] * a[1], (a[0] + a[0]) * a[1]


def tl(i, n=1):
    return slice(128 * i, 128 * (i + n))


def rs(a, n):
    return slice(a, a + n)


def _kernel(x_hbm, are_h, aim_h, bre_h, bim_h, cre_h, cim_h, ldt_h, dsk_h, wg_h, wu_h, wd_h,
            big_h, sm_h, o_hbm,
            x_v, par_v, ldt_v, dsk_v, wg_v, wu_v, wd_v, big_v, sm_v, coef_s, zw_s, xn_u, xa_u, ha_u,
            wt_u, wdt_u, u_s, xs_u, es_u, kc_s, kw_s, kd_s, y_u, o_s, dum_v, sems):
    off = _consts()[0]
    xn_s, xa_s, ha_s, wt_s, wdt_s, xs_s, es_s, y_s, big_s, sm_s = [
        _Packed(r) for r in (xn_u, xa_u, ha_u, wt_u, wdt_u, xs_u, es_u, y_u, big_v, sm_v)]
    x_u, wg_u, wu_u, wd_u, o_u = [_Words(r) for r in (x_v, wg_v, wu_v, wd_v, o_s)]
    AL = slice(None)
    nsem = [0]

    def grp(pairs):
        nsem[0] += 1
        return [pltpu.make_async_copy(a, b, sems.at[nsem[0] - 1]) for a, b in pairs]

    def cf(r0, n):
        return pltpu.bitcast(big_v[rs(off["F32"] + r0, n), :], f32)

    def mk(paced=True):
        c = _Ctx()
        c.never = (sm_v[0:8, :] != 0) if paced else None
        c.tok = c.xt = None
        c.cnt = 0
        return c

    def tie(c, v, tok):
        if tok is None or c.never is None:
            return v
        if tok.dtype != v.dtype:
            tok = pltpu.bitcast(tok, v.dtype)
        h = jnp.where(c.never, tok, v[:, :128])
        return h if v.shape[1] == 128 else _cat([h, v[:, 128:]], 1)

    def a0(c, ct, nc):
        cs = tl(ct)
        dt = jnp.exp(ldt_v[...].astype(f32).reshape(1, D)[:, cs]).astype(bf16).astype(f32)
        outs = [[], [], [], []]
        k0 = None
        toks = [c.tok] * nc
        for i in range(N // 8):
            ld = lambda q: par_v[q, 8 * i:8 * i + 8, cs].astype(f32)
            tk = toks[i % nc]
            zr, zi = _cis(jnp.exp(dt * ld(0)), tie(c, dt * ld(1), tk))
            cb = _cmul((ld(4), ld(5)), (tie(c, ld(2), tk), tie(c, ld(3), tk)))
            wr, wi = dt * cb[0], dt * cb[1]
            k0 = wr if k0 is None else k0 + wr
            toks[i % nc] = zr
            for o, v in zip(outs, (zr, zi, wr, wi)):
                o.append(v)
        c.tok = toks[-1]
        coef_s[:, cs] = jnp.broadcast_to(
            jnp.sum(k0, axis=0, keepdims=True) + dsk_v[...].astype(f32).reshape(1, D)[:, cs], (8, 128))
        hi = [outs[0][16:] * 2, outs[1][16:] * 2, [-v for v in outs[3][16:]] + outs[2][16:], outs[2][16:] + outs[3][16:]]
        for q in range(4):
            for h, v in enumerate((_cat(outs[q][:16], 0).T, _cat(hi[q], 0).T)):
                zw_s[q, cs, tl(h)] = v
                c.xt = v[120:128] if c.xt is None else c.xt + v[120:128]

    def ln(c, t, toks):
        for i in range(8):
            eo = ([], [])
            for g in range(2):
                wr = rs(128 * t + 16 * i + 8 * g, 8)
                for hh, xx in enumerate(_even_odd(x_u[wr, AL])):
                    ci = (4 * i + 2 * g + hh) % len(toks)
                    xx = tie(c, xx, toks[ci])
                    xc = xx - jnp.sum(xx, axis=1, keepdims=True) * (1.0 / D)
                    var = jnp.sum(xc * xc, axis=1, keepdims=True) * (1.0 / D)
                    xn = xc * jax.lax.rsqrt(var + 1e-5)
                    toks[ci] = xn[:, :128]
                    eo[hh].append(xn)
            top, bot = _cat(eo[0], 0), _cat(eo[1], 0)
            xn_s[rs(RB * t + 16 * i, 16), AL] = top
            xn_s[rs(RB * t + 128 + 16 * i, 16), AL] = bot
            a11, a12, a21, a22 = top[:, 0:256], top[:, 256:512], bot[:, 0:256], bot[:, 256:512]
            for q, v in enumerate((a11 + a22, a21 + a22, a11 + a12, a21 - a11, a12 - a22)):
                xa_s[rs(128 * t + 16 * i, 16), tl(2 * q, 2)] = v

    def bcomb(c, src, dst, kw, n1, dcol, srow):
        for i in range(kw // 8):
            ws = [tie(c, src[rs(srow(h, i), 8), tl(n)], c.tok) for h in range(2) for n in (n1, n1 + 1)]
            q = [_even_odd(w) for w in ws]
            res = []
            for p in range(2):
                b11, b12, b21, b22 = (v[p] for v in q)
                res.append((b11 + b22, b12 - b22, b21 - b11, b11 + b12, b21 + b22))
            pks = [_zip2(res[0][j], res[1][j]) for j in range(5)] + [ws[0], ws[3]]
            for j, pk in enumerate(pks):
                dst[rs(j * kw + 8 * i, 8), tl(dcol)] = pk
            c.tok = res[0][1] + (res[0][0] + pltpu.bitcast(pks[4], f32))

    def wcomb(c, ck):
        for m, src in enumerate((wg_u, wu_u)):
            bcomb(c, src, wt_u, 128, 2 * ck, 2 * ck + m, lambda h, i: 128 * h + 8 * i)
            for i in range(8):
                ws = [tie(c, src[rs(256 + 8 * i, 8), tl(n)], c.tok) for n in (2 * ck, 2 * ck + 1)]
                q = [_even_odd(w) for w in ws]
                c.tok = q[0][0] + q[1][0]
                for j, w in enumerate((_zip2(c.tok, q[0][1] + q[1][1]), ws[0], ws[1])):
                    wt_u[rs(896 + 64 * j + 8 * i, 8), tl(2 * ck + m)] = w

    def wdcomb(c, pr):
        srow = lambda h, i: 128 * (i // 8) + 64 * h + 8 * (i % 8)
        bcomb(c, wd_u, wdt_u, 384, 2 * pr, pr, srow)
        for i in range(48):
            w = tie(c, wd_u[rs(srow(pr, i), 8), tl(4)], c.tok)
            wdt_u[rs(7 * 384 + 8 * i, 8), tl(pr)] = w
            c.tok = pltpu.bitcast(w, f32) + 1.0

    def xe(c, o):
        lo64, slo = sm_v[16:24, :] != 0, sm_v[24:32, :] != 0
        rolled = {}

        def roll4(v):
            if id(v) not in rolled:
                rolled[id(v)] = (v, pltpu.roll(v, 4, 0))
            return rolled[id(v)][1]

        def mix(a, b, g):
            return tuple(jnp.where(slo, u, roll4(v)) if g == 0 else jnp.where(slo, roll4(u), v) for u, v in zip(a, b))

        def tiec(v, tok):
            return tuple(tie(c, u, tok) for u in v)

        l01 = jnp.where(lo64, 1.0, 0.0).astype(f32)
        prep = []
        tok = c.tok
        for h in range(2):
            z = tiec((zw_s[0, rs(8 * o, 8), tl(h)], zw_s[1, rs(8 * o, 8), tl(h)]), tok)
            w = (zw_s[2, rs(8 * o, 8), tl(h)], zw_s[3, rs(8 * o, 8), tl(h)])
            pw = {1: z}
            e = 1
            while e < 512:
                pw[2 * e] = _csq(pw[e])
                e *= 2
                if e == 2:
                    wz = _cmul(w, z)
                if e == 8:
                    wz5 = _cmul(wz, pw[4])
            p772 = _cmul(_cmul(pw[256], pw[4]), pw[512])
            er, ei = pw[128]
            if h == 0:
                one, eb = (jnp.ones((8, 128), f32), jnp.zeros((8, 128), f32)), (er, -ei)
            else:
                one, eb = (1.0 - l01, l01), (jnp.where(lo64, ei, er), jnp.where(lo64, er, -ei))
            prep.append((z, wz, wz5, pw[256], p772, pw[8], one, eb))
            if c.xps:
                tok = p772[0]
        tok = p772[0]
        for g in range(2):
            def put(ref, n, lst, h):
                i = len(lst) - 2
                if i % 2 == 0:
                    b0 = (2 * (o % XR) + g) * 8 * n + 8 * i
                    for q, cb in ([(0, 0), (1, 1)] if h == 0 else [(1, 2)]):
                        ref[rs(b0, 16), tl(cb)] = _cat([lst[i][q], lst[i + 1][q]], 0)

            def xseg(h, tok):
                z, wz, wz5, p256, p772 = prep[h][:5]
                xs = [tiec(mix(wz, wz5, g), tok)]
                a1 = mix(z, z, g)
                a256 = am = None
                for src in (0, 1, 2, 1, 3, 5, 6, 7, 8):
                    if len(xs) == 3:
                        a256 = mix(p256, p256, g)
                    if len(xs) == 6:
                        am = mix(p772, p256, g)
                    xs.append(_cmul(xs[src], a1 if len(xs) < 4 else (am if len(xs) == 8 else a256)))
                    put(xs_s, 10, xs, h)
                return xs[-1][1]

            def eseg(hs, tok):
                es, a8 = {}, {}
                for h in hs:
                    p8, one, eb = prep[h][5:]
                    a8[h] = mix(p8, p8, g)
                    es[h] = [tiec(tuple(jnp.where(slo, u, roll4(v) if g == 0 else v) for u, v in zip(one, eb)), tok)]
                if 1 in hs:
                    ra, rb = a8[1][0] + a8[1][0], a8[1][0] * a8[1][0] + a8[1][1] * a8[1][1]
                for v in range(15):
                    for h in hs:
                        if h == 0 or v == 0:
                            es[h].append(_cmulc(es[h][-1], a8[h]))
                        else:
                            es[h].append((None, ra * es[h][-1][1] - rb * es[h][-2][1]))
                        put(es_s, 16, es[h], h)
                return es[hs[0]][-1][1]

            tok = xseg(0, tok)
            tok = eseg([1], eseg([0], tok)) if (c.xs2 and (2 * o + g) % c.xs2 == 0) else eseg([0, 1], tok)
            tok = xseg(1, tok)
        c.tok = tok

    def c2(c, unit):
        ct, p = divmod(unit, 8)
        ys, gs = {}, {}
        for cl in (0, 2, 1, 3):
            rws = rs(64 * cl + 8 * p, 8)
            pos = cl in (0, 3)

            def kpart(pt, s):
                ht = lambda q: cf(off["T", pt[0]] + 256 * q + 64 * cl + 8 * p, 8)
                kd = lambda q: kd_s[ct, _KD[pt, q] + (p % (16 // pt[0]) if q in range(6) else 0)]
                half = pt[3] - pt[2] == 256
                if s == 0:
                    kv = ht(0) * kd(4) + ht(1) * kd(5)
                    return kv if not half else (kv + ht(2) * kd("b") if pos else kv - ht(2) * kd("b"))
                q = (s - 1) ^ (not pos)
                kv, tv = ht(0) * kd(q) + ht(1) * kd(2 + q), ht(2) * kd("a-b" if half and q else "a+b")
                return kv - tv if s == 1 else kv + tv

            k1, ri = None, {}
            for s in range(3):
                U, K, out = [], [], []
                for i in range(NS):
                    U.append(u_s[ct, 0, i, rws, :] + u_s[ct, 1, i, rws, :] if s == 0 else u_s[ct, s - 1, i, rws, :])
                    ks = [kpart(pt, s) for pt in _PARTS if pt[1] == i]
                    if i < 3:
                        ks.append((kw_s[ct, 0, i, rws, :] + kw_s[ct, 1, i, rws, :]) * (-0.5) if s == 0
                                  else kw_s[ct, s - 1, i, rws, :])
                    K.append(ks[0] if len(ks) == 1 else ks[0] + ks[1])
                    ms = list(range(1, i)) + ([0, i] if i else [0])
                    a = tie(c, k1[i] if s else K[ms[0]] * U[i - ms[0]], c.tok)
                    ms = ms if s else ms[1:]
                    while ms:
                        c.cnt += 1
                        pr = K[ms[0]] * U[i - ms[0]]
                        if c.cnt % c.ps[1] < c.ps[0] and len(ms) > 1 and (c.jit or not (s == 2 and cl == 3)):
                            pr = pr + K[ms[1]] * U[i - ms[1]]
                            ms = ms[1:]
                        ms = ms[1:]
                        a = a + pr
                    c.tok = a
                    out.append(a)
                    if s == 2 and cl >= 2:
                        yr, yi, zr, zi = ys[cl - 2][2][i], ys[cl - 2][1][i], a, ri[1][i]
                        g = (yr + zr, yi - zi, yr - zr, yi + zi)
                        if cl == 2:
                            gs[i] = g
                            c.tok = a if c.jit else g[2]
                        else:
                            e = gs[i]
                            hs = ((e[0] + g[0], e[1] - g[1]), (e[2] - g[3], e[3] - g[2]),
                                  (e[0] - g[0], e[1] + g[1]), (e[2] + g[3], e[3] + g[2]))
                            for q, h in enumerate(hs):
                                y_s[rs(512 * ct + 128 * q + 16 * p, 16), tl(i)] = _cat(h, 0)
                            c.tok = a if c.jit else hs[3][1] + hs[0][0]
                if s == 0:
                    k1 = out
                else:
                    ri[s] = out
            ys[cl] = ri

    queue = []

    def hook():
        if queue:
            queue.pop(0)()

    def ffn1(t, ck, strassen=True):
        top, bot = rs(RB * t, 128), rs(RB * t + 128, 128)
        if strassen:
            cw = tl(2 * ck, 2)
            sa = lambda q: xa_s[rs(128 * t, 128), tl(2 * q, 2)]
            tb = lambda q: wt_s[rs(256 * q, 256), cw]
            tk, k3a, k3b = (wt_s[rs(1792 + 128 * j, 128), cw] for j in range(3))
            m4 = _dot(xn_s[bot, tl(2, 2)], tb(2))
            hook()
            m2 = _dot(_cat([sa(1), xn_s[bot, tl(4)]], 1), _cat([tb(5), k3a], 0))
            c21 = m2 + m4
            hook()
            m5 = _dot(_cat([sa(2), xn_s[top, tl(4)]], 1), _cat([tb(6), k3b], 0))
            hook()
            m3 = _dot(xn_s[top, tl(0, 2)], tb(1))
            c12 = m3 + m5
            hook()
            m1 = _dot(sa(0), tb(0))
            hook()
            m7 = _dot(_cat([sa(4), xn_s[top, tl(4)]], 1), _cat([tb(4), tk], 0))
            hook()
            m6 = _dot(_cat([sa(3), xn_s[bot, tl(4)]], 1), _cat([tb(3), tk], 0))
            c11, c22 = m7 + (m1 + (m4 - m5)), m6 + (m1 + (m3 - m2))
        else:
            xn = xn_s[rs(RB * t, RB), AL]
            r1 = _dot(xn, _cat([wg_v[:, tl(2 * ck)], wu_v[:, tl(2 * ck)]], 1))
            r2 = _dot(xn, _cat([wg_v[:, tl(2 * ck + 1)], wu_v[:, tl(2 * ck + 1)]], 1))
            c11, c21, c12, c22 = r1[:128], r1[128:], r2[:128], r2[128:]
        h11, h12, h21, h22 = (v[:, :128] * v[:, 128:] for v in (c11, c12, c21, c22))
        for q, v in enumerate((h11, h12, h21, h22, h11 + h22, h21 + h22, h11 + h12, h21 - h11, h12 - h22)):
            ha_s[rs(128 * t, 128), tl(6 * q + ck)] = v
        return c21[0:8, 0:128]

    def ufwd(t):
        for c0, n in ((0, 2), (2, 2), (4, 1)):
            e = _dot(sm_s[64:320, AL], xn_s[rs(RB * t, 128), tl(c0, n)])
            o = _dot(sm_s[320:576, AL], xn_s[rs(RB * t + 128, 128), tl(c0, n)])
            for j in range(n):
                er, ei, or_, oi = e[:128, tl(j)], e[128:, tl(j)], o[:128, tl(j)], o[128:, tl(j)]
                u_s[c0 + j, 0, t, 0:128], u_s[c0 + j, 0, t, 128:256] = er + or_, er - or_
                u_s[c0 + j, 1, t, 0:128], u_s[c0 + j, 1, t, 128:256] = ei + oi, oi - ei
            if c0 == 0:
                yield

    def kmm(o):
        lane = jax.lax.broadcasted_iota(i32, (8, 128), 1)
        sub = jax.lax.broadcasted_iota(i32, (8, 128), 0)
        slo = sub < 4
        res = [_nt(xs_s[rs(80 * q, 80), AL], es_s[rs(128 * q, 128), AL]) for q in (2 * (o % XR), 2 * (o % XR) + 1)]
        dk = (lane - sub) & 3

        def merge(r, vs):
            out = None
            for k in reversed(range(len(vs))):
                src = r[8 * vs[k]:8 * vs[k] + 8, :]
                if k:
                    src = pltpu.roll(src, k, 1)
                out = src if out is None else jnp.where(dk == k, src, out)
            return out

        def derot(x):
            x = jnp.where((sub & 1) == 1, pltpu.roll(x, 127, 1), x)
            return jnp.where((sub & 2) == 2, pltpu.roll(x, 126, 1), x)

        ts = []
        for vs, sh in (([0, 1, 2, 3], 1), ([4, 5, 6, 7], 2), ([8, 9], 2)):
            a, b = merge(res[0], vs), merge(res[1], vs)
            a, b = jnp.where(slo, a, pltpu.roll(b, 4, 0)), pltpu.roll(jnp.where(slo, pltpu.roll(a, 4, 0), b), sh, 1)
            m = (dk & sh) == 0
            ts += [jnp.where(m, a, b), jnp.where(m, b, a)]
        for i in range(5):
            kc_s[i, rs(8 * o, 8), :] = derot(ts[i])

    def kfwd(ct):
        kt = lambda tau: kc_s[tau, tl(ct), :].astype(bf16)
        kv = {}
        for tau, lg in _SEL.items():
            v = _nt(big_s[rs(off["D", tau], off["Dn", tau]), AL], kt(tau))
            kv.update({lag: v[rs(8 * j, 8)] for j, lag in enumerate(lg)})
            r0 = 16 * ((len(lg) + 1) // 2)
            for pt in [p for p in _PARTS if p[0] == {3: 4, 4: 8}.get(tau)]:
                st, w, p0, p1 = pt
                n = 16 // st
                d = [[v[rs(r0 + 8 * (n * q + j), 8)] for j in range(n)] for q in range(4)]
                r0 += 32 * n
                vl, vr = kv[256 * (w - 1) + p0], kv[256 * (w - 1) + p1]
                if 256 * (w - 1) + p0 not in lg:
                    hv = vl * 0.5
                    d[0], d[1] = [x - hv for x in d[0]], [x + hv if p0 else x - hv for x in d[1]]
                d += [[(x + y) * (-0.5) for x, y in zip(d[q], d[q + 1])] for q in (0, 2)]
                for q in range(6):
                    for j in range(n):
                        kd_s[ct, _KD[pt, q] + j] = d[q][j]
                if p1 - p0 == 512:
                    kd_s[ct, _KD[pt, "a+b"]] = vl + vr
                else:
                    a, b = (vr, -vl) if p0 else (vl, vr)
                    kd_s[ct, _KD[pt, "a+b"]], kd_s[ct, _KD[pt, "a-b"]], kd_s[ct, _KD[pt, "b"]] = a + b, a - b, b
        yield
        for cb in range(2):
            od, ev = (_nt(big_s[rs(off["B0", t] + 128 * cb, 128), AL], kt(t)) for t in (0, 1))
            sm, df = ev + od, ev - od
            for cl, (e0, f0) in ((cb, (sm[:64], sm[64:])), (cb + 2, (df[64:], df[:64]))):
                pos, rw = cl in (0, 3), rs(64 * cl, 64)
                v = _nt(big_s[rs(off["B1"] + 128 * cl, 128), AL], kt(2)) + cf(128 * cl, 128) * _cat([kv[256]] * 16, 0)
                e1, f1 = v[:64], v[64:]
                kw_s[ct, 0, 0, rw], kw_s[ct, 1, 0, rw] = (f0, -e0) if pos else (-f0, e0)
                kw_s[ct, 0, 1, rw], kw_s[ct, 1, 1, rw] = (e0 + f1, f0 - e1) if pos else (e0 - f1, f0 + e1)
                kw_s[ct, 0, 2, rw], kw_s[ct, 1, 2, rw] = e1, f1
            yield

    def inv(ct, t):
        y = [_dot(big_s[rs(off["I", q], 64), AL], y_s[rs(512 * ct + 128 * q, 128), tl(t)]) for q in range(4)]
        return _zip2(y[0], y[2]), _zip2(y[1], y[3])

    def finish(ct, t, dt_, db_):
        y = inv(ct, t)
        xs = _even_odd(x_u[rs(128 * t, 128), tl(ct)])
        res = []
        for h, dn in enumerate((dt_, db_)):
            yy = pltpu.bitcast(y[h], bf16).astype(f32)
            xn = xn_s[rs(RB * t + 128 * h, 128), tl(ct)].astype(f32)
            res.append(xs[h] + (xn * coef_s[0:1, tl(ct)] + dn) + yy)
        o_u[rs((ct * L + RB * t) // 2, 128), AL] = _zip2(*res)
        c_out[ct * NS + t].start()

    pend = {}

    def flush(ct, t):
        finish(ct, t, *pend.pop((ct, t)))

    def down4(t):
        dn = _dot(_cat([ha_s[rs(128 * t, 128), 0:1536], ha_s[rs(128 * t, 128), 1536:3072]], 0),
                  _cat([wdt_s[5376:6144, tl(0)], wdt_s[5376:6144, tl(1)]], 0))
        pend[4, t] = (dn[:128], dn[128:])

    def down_pair(pr, t):
        m = {}
        for k, (a, b) in ((1, (4, 0)), (4, (3, 2)), (5, (6, 6)), (7, (8, 4)), (2, (5, 5)), (3, (0, 1)), (6, (7, 3))):
            m[k] = _dot(ha_s[rs(128 * t, 128), tl(6 * a, 6)], wdt_s[rs(768 * b, 768), tl(pr)])
            if k == 2:
                pend[2 * pr, t] = (m[7] + m[1] + m[4] - m[5], m[2] + m[4])
            if k == 6:
                pend[2 * pr + 1, t] = (m[3] + m[5], m[6] + m[1] - m[2] + m[3])
            yield

    pars = (are_h, aim_h, bre_h, bim_h, cre_h, cim_h)
    par = lambda a, n: [(p.at[:, tl(a, n)], par_v.at[i, :, tl(a, n)]) for i, p in enumerate(pars)]
    xr = lambda a, b: [(x_hbm.at[a * RB:b * RB], x_v.at[a * RB:b * RB])]
    wch = lambda a, n: [(h.at[:, tl(2 * a, 2 * n)], v.at[:, tl(2 * a, 2 * n)]) for h, v in ((wg_h, wg_v), (wu_h, wu_v))]
    dum = lambda i: [(sm_h.at[0:8], dum_v.at[8 * i:8 * i + 8])]
    G = [grp(p) for p in (
        xr(0, 1), [(sm_h, sm_v)] + xr(1, 2), wch(0, 1), wch(1, 1) + xr(2, 3),
        wch(2, 1) + xr(3, 4) + par(0, 1) + [(ldt_h, ldt_v), (dsk_h, dsk_v)], par(1, 1) + wch(3, 3),
        par(2, 3) + xr(4, 8), [(big_h, big_v), (wd_h, wd_v)], dum(0), dum(1), dum(2))]
    c_out = grp([(o_s.at[rs(ct * L + RB * t, RB)], o_hbm.at[rs(RB * t, RB), tl(ct)])
                 for ct in range(NCT) for t in range(NS)])

    def wait(cs):
        for cc in cs:
            cc.wait()

    def run_all(gen):
        for _ in gen:
            pass

    def part(c, main=(), km=(), uf=(), kf=(), wc=(), wdc=(), lns=(), a0s=(), xes=(), c2s=(),
             late=None, nw=4, nk=None, xps=1, ps=(1, 1), xs2=0, nc=2, jit=0, wcj=(), fine=1):
        c.xps, c.ps, c.xs2, c.jit = xps, ps, xs2, jit
        if wcj:
            keep = c.tok, c.never
            c.tok, c.never = None, sm_v[288:296, :] != 0
            for ck in wcj:
                wcomb(c, ck)
            c.tok, c.never = keep
        for ck in wc:
            wcomb(c, ck)
        for pr in wdc:
            wdcomb(c, pr)
        for o in xes:
            xe(c, o)
        for un in c2s:
            c2(c, un)
        extra = []
        for gen, n in [(ufwd(t), 2) for t in uf] + [(kfwd(ct), 3) for ct in kf]:
            extra += [functools.partial(next, gen, None)] * n
        nm, kms, mt = len(main), list(km), []
        nkk = nk if nk is not None else nm - 1
        for i, fn in enumerate(main):
            if i < nkk:
                queue.extend(functools.partial(kmm, o) for o in kms[i * len(kms) // nkk:(i + 1) * len(kms) // nkk])
            queue.extend(extra[i * len(extra) // nm:(i + 1) * len(extra) // nm])
            while len(queue) > (6 if fine else 0):
                hook()
            mt.append(fn())
            while queue:
                hook()
        if a0s or lns:
            keep = c.tok, c.never
            c.tok, c.never = (None if late is None else mt[late]), sm_v[8:16, :] != 0
            for ct in a0s:
                a0(c, ct, nc)
            toks = [c.xt if a0s else c.tok] * nw
            for q in range(1, nw if toks[0] is not None else 0):
                toks[q] = functools.reduce(lambda a, _: a + 1.0, range(20), toks[q - 1])
            for t in lns:
                ln(c, t, toks)
            c.tok, c.never = keep

    def block(waits, *parts, end=()):
        def run():
            wait(waits)
            c = mk()
            for p in (parts[0]() if callable(parts[0]) else parts):
                part(c, **p)
            wait(end)
        return run

    for g in G:
        for cc in g:
            cc.start()
    flag = jax.lax.fori_loop(0, 3, lambda i, a: a + i, 0)
    wait(G[0])
    ln(mk(False), 0, [None])

    def p1():
        wait(G[1])
        run_all(ufwd(0))
        ln(mk(False), 1, [None])
        run_all(ufwd(1))

    R, P = range, functools.partial
    it = [P(ffn1, t, ck) for t, ck in ([(t, ck) for t in (2, 3) for ck in R(3)] + [(t, ck) for t in R(4) for ck in R(3, 6)]
                                       + [(t, ck) for t in R(4, 8) for ck in R(6)])]

    def pairs(pr, inline):
        out = []
        fl = lambda ct, t: [P(flush, ct, t)] if inline and t >= 0 else []
        for t in R(NS):
            d = [P(next, down_pair(pr, t), None)] * 7
            out += d[:1] + fl(2 * pr, t - 1) + d[1:3] + fl(2 * pr + 1, t - 1) + d[3:]
        return out[:-2] + fl(2 * pr, NS - 1) + out[-2:] + fl(2 * pr + 1, NS - 1)

    def yparts():
        m = pairs(0, True)
        return [dict(main=m[:56], km=R(64, 80), nk=40, c2s=R(16, 27), ps=(0, 1), fine=0),
                dict(main=m[56:], kf=[4], fine=0)]

    def zparts():
        m = pairs(1, False)
        for t in R(NS):
            m += [P(down4, t)] + [P(flush, ct, t) for ct in (2, 3) if t < 6] + [P(flush, 4, t)]
            if 3 <= t <= 6:
                m += [P(flush, 2 + (t + 1) % 2, 6 + (t - 3) // 2)]
        return [dict(main=m, c2s=R(27, 40), ps=(2, 3), jit=1)]

    blocks = [
        p1,
        block(G[2], dict(main=[P(ffn1, 0, 0, False), P(ffn1, 1, 0)], wcj=[0])),
        block(G[3], dict(main=[P(ffn1, 0, 1, False), P(ffn1, 1, 1)], wcj=[1], lns=[2], nw=5)),
        block(G[4], dict(main=it[0:1] + [P(ffn1, 0, 2), P(ffn1, 1, 2)] + it[1:2], uf=[2], wcj=[2], a0s=[0], lns=[3], nc=1, nw=8)),
        block(G[5], dict(main=it[2:6], uf=[3], wc=[3, 4, 5], xes=R(0, 10), a0s=[1], xps=0, nc=3)),
        block(G[6], dict(main=it[6:18], km=R(0, 10), xes=R(10, 32), lns=R(4, 8), a0s=[2, 3], late=5, nk=5,
                         nw=8, xps=0, nc=2)),
        block(G[7], dict(main=it[18:24], km=R(10, 32), nk=5, uf=R(4, 8), wdc=[0, 1], xes=R(32, 64),
                         xs2=2),
              dict(main=it[24:28], kf=[0, 1], a0s=[4], late=2, nc=1)),
        block(G[8], dict(main=it[28:40], km=R(32, 64), nk=6, xes=R(64, 80), xs2=2, c2s=R(0, 16), ps=(1, 3)),
              dict(main=it[40:42], kf=[2, 3])),
        block(G[9], yparts),
        block(G[10], zparts, end=c_out),
    ]
    for i, fn in enumerate(blocks):
        pl.when(flag > -i)(fn)


@jax.jit
def pallas_parallel_sum__ssm_conv_s4__glu_gated_bilinear__prompt_kernel(A_u, A_A_re, A_A_im, A_B_re, A_B_im, A_C_re, A_C_im, A_log_dt, A_Dskip, B_x, B_w_gate, B_w_up, B_w_down):
    _, big, small = _consts()
    hbm = pl.BlockSpec(memory_space=pltpu.HBM)
    out = pl.pallas_call(
        _kernel,
        in_specs=[hbm] * 14,
        out_specs=hbm,
        out_shape=jax.ShapeDtypeStruct((L, D), bf16),
        scratch_shapes=[
            pltpu.VMEM((L, D), bf16),
            pltpu.VMEM((6, N, D), bf16),
            pltpu.VMEM((D,), bf16), pltpu.VMEM((D,), bf16),
            pltpu.VMEM((D, F), bf16), pltpu.VMEM((D, F), bf16), pltpu.VMEM((F, D), bf16),
            pltpu.VMEM(big.shape, u32), pltpu.VMEM(small.shape, u32),
            pltpu.VMEM((8, D), f32),
            pltpu.VMEM((4, D, 256), f32),
            pltpu.VMEM((L // 2, D), u32),
            pltpu.VMEM((L // 4, 1280), u32),
            pltpu.VMEM((L // 4, 9 * 768), u32),
            pltpu.VMEM((1088, F), u32),
            pltpu.VMEM((8 * 384, 256), u32),
            pltpu.VMEM((NCT, 2, NS, 256, 128), f32),
            pltpu.VMEM((2 * XR * 40, 384), u32),
            pltpu.VMEM((2 * XR * 64, 384), u32),
            pltpu.VMEM((5, D, 128), f32),
            pltpu.VMEM((NCT, 2, 3, 256, 128), f32),
            pltpu.VMEM((NCT, _KD["n"], 8, 128), f32),
            pltpu.VMEM((NCT * 256, NS * 128), u32),
            pltpu.VMEM((NCT * L, 128), bf16),
            pltpu.VMEM((24, 128), u32),
            pltpu.SemaphoreType.DMA((12,)),
        ],
        compiler_params=pltpu.CompilerParams(vmem_limit_bytes=110 * 1024 * 1024),
    )(A_u.reshape(L, D), A_A_re.T, A_A_im.T, A_B_re.T, A_B_im.T, A_C_re.T, A_C_im.T, A_log_dt, A_Dskip,
      B_w_gate, B_w_up, B_w_down, jnp.asarray(big), jnp.asarray(small))
    return out.reshape(1, L, D)
```
